```python
import jax
import jax.numpy as jnp

def _softmax(x, axis=-1):
    return jax.nn.softmax(x, axis=axis)

def _gelu(x):
    return jax.nn.gelu(x, approximate=True)

def _silu(x):
    return jax.nn.silu(x)

def _sigmoid(x):
    return jax.nn.sigmoid(x)

def _layernorm(x, axis=-1, eps=1e-05):
    m = jnp.mean(x, axis=axis, keepdims=True)
    v = jnp.var(x, axis=axis, keepdims=True)
    return (x - m) / jnp.sqrt(v + eps)

def _scatter_add(tgt, idx, src, axis=0):
    return tgt.at[idx].add(src)

def _segment_sum(src, seg, n):
    return jax.ops.segment_sum(src, seg, n)

class _Rng:

    def __init__(self, key):
        self._k = key

    def _next(self):
        self._k, sub = jax.random.split(self._k)
        return sub

    def normal(self, shape):
        return jax.random.normal(self._next(), shape, dtype=jnp.bfloat16)

    def randint(self, lo, hi, shape):
        return jax.random.randint(self._next(), shape, lo, hi, dtype=jnp.int32)

    def uniform(self, shape, lo=0.0, hi=1.0):
        return jax.random.uniform(self._next(), shape, jnp.bfloat16, lo, hi)

    def permutation(self, n):
        return jax.random.permutation(self._next(), n)
kernel_name = 'parallel_sum__memory_aug_recurrent_mem_tr__moe_arch_mod__prompt'

def setup_inputs():
    _rng = _Rng(jax.random.key(int.from_bytes(__import__("os").urandom(4), "little")))
    _w = lambda a: (lambda t: t.astype(jnp.bfloat16) if jnp.issubdtype(t.dtype, jnp.floating) else t)(jnp.asarray(a))

    def _A_setup():
        B, S, Dm = (1, 2048, 1024)
        H, Dh = (32, 128)
        M, seg = (8, 32)
        seg = min(seg, S)
        S = S // seg * seg
        return {'x': _w((lambda *s: _rng.normal(s) * 0.05)(B, S, Dm)), 'mem0': _w((lambda *s: _rng.normal(s) * 0.05)(B, M, Dm)), 'Wq': _w((lambda *s: _rng.normal(s) * 0.05)(Dm, H, Dh) * Dm ** (-0.5)), 'Wk': _w((lambda *s: _rng.normal(s) * 0.05)(Dm, H, Dh) * Dm ** (-0.5)), 'Wv': _w((lambda *s: _rng.normal(s) * 0.05)(Dm, H, Dh) * Dm ** (-0.5)), 'Wo': _w((lambda *s: _rng.normal(s) * 0.05)(H, Dh, Dm) * (H * Dh) ** (-0.5)), 'seg_len': seg}
    _A_in = _A_setup()

    def _B_setup():
        B, S, D, F, C = (1, 2048, 1024, 3584, 2)
        return {'x': _w((lambda *s: _rng.normal(s) * 0.05)(B, S, D)), 'w_r': _w((lambda *s: _rng.normal(s) * 0.05)(D)), 'w_gate': _w((lambda *s: _rng.normal(s) * 0.05)(D, F)), 'w_up': _w((lambda *s: _rng.normal(s) * 0.05)(D, F)), 'w_down': _w((lambda *s: _rng.normal(s) * 0.05)(F, D))}
    _B_in = _B_setup()
    return {'A_x': _A_in['x'], 'A_mem0': _A_in['mem0'], 'A_Wq': _A_in['Wq'], 'A_Wk': _A_in['Wk'], 'A_Wv': _A_in['Wv'], 'A_Wo': _A_in['Wo'], 'A_seg_len': _A_in['seg_len'], 'B_x': _B_in['x'], 'B_w_r': _B_in['w_r'], 'B_w_gate': _B_in['w_gate'], 'B_w_up': _B_in['w_up'], 'B_w_down': _B_in['w_down']}

def reference(A_x, A_mem0, A_Wq, A_Wk, A_Wv, A_Wo, A_seg_len, B_x, B_w_r, B_w_gate, B_w_up, B_w_down):

    def _A_ref(x, mem0, Wq, Wk, Wv, Wo, seg_len):
        B, S, Dm = x.shape
        H, Dh = (Wq.shape[1], Wq.shape[2])
        M = mem0.shape[1]
        scale = Dh ** (-0.5)
        n_seg = S // seg_len
        L = M + seg_len
        idx = jnp.arange(L)
        mask = (idx[:, None] < M) | (idx[:, None] >= idx[None, :])
        mem = mem0
        outs = []
        for s in range(n_seg):
            xs = x[:, s * seg_len:(s + 1) * seg_len, :].copy()
            h = jnp.concatenate([mem, xs], axis=1)
            q = jnp.einsum('btd,dhe->bhte', h, Wq)
            k = jnp.einsum('btd,dhe->bhte', h, Wk)
            v = jnp.einsum('btd,dhe->bhte', h, Wv)
            scores = jnp.einsum('bhqe,bhke->bhqk', q, k) * scale
            scores = jnp.where(mask[None, None], scores, -1000000000.0)
            p = _softmax(scores, axis=-1)
            o = jnp.einsum('bhqk,bhke->bhqe', p, v)
            o = jnp.einsum('bhte,hed->btd', o, Wo)
            mem = o[:, :M, :].copy()
            outs.append(o[:, M:, :])
        return jnp.concatenate(outs, axis=1)

    def _B_ref(x, w_r, w_gate, w_up, w_down):
        B, S, D = x.shape
        C = 2
        r = x @ w_r
        idx = jnp.argsort(-r, axis=-1)[:, :C]
        idx_e = jnp.repeat(idx.reshape(B, C, 1), D, axis=2)
        x_sel = jnp.take_along_axis(x, idx_e, axis=1)
        g = _silu(x_sel @ w_gate)
        u = x_sel @ w_up
        y = g * u @ w_down
        r_sel = _sigmoid(jnp.take_along_axis(r, idx, axis=1))
        y = y * r_sel.reshape(B, C, 1)
        b_off = (jnp.arange(B) * S).reshape(B, 1)
        flat_idx = (idx + b_off).reshape(B * C)
        zero = (x * 0.0).reshape(B * S, D)
        upd = _scatter_add(zero, flat_idx, y.reshape(B * C, D), axis=0)
        return x + upd.reshape(B, S, D)
    x = A_x
    xn = _layernorm(x, axis=-1)
    return x + _A_ref(xn, A_mem0, A_Wq, A_Wk, A_Wv, A_Wo, A_seg_len) + _B_ref(xn, B_w_r, B_w_gate, B_w_up, B_w_down)
```

```python
import functools
import jax
import jax.numpy as jnp
import numpy as np
import jax.experimental.pallas as pl
import jax.experimental.pallas.tpu as pltpu

F32, BF16, U32, I32 = jnp.float32, jnp.bfloat16, jnp.uint32, jnp.int32
NT = (((1,), (1,)), ((), ()))


def _rnd(v):
    return v.astype(BF16).astype(F32)


def _dot(a, b):
    return jnp.dot(a, b, preferred_element_type=F32)


def make_kernel(S, D, H, Dh, M, SEG, F, nsteps=None):
    assert (Dh, M, SEG) == (128, 8, 32) and D % 128 == 0 and F % 128 == 0 and S % 64 == 0
    KD, NF = D // 128, F // 128
    L = M + SEG
    DC = 128
    NCH = D // DC
    NST = 4
    scale = Dh ** -0.5
    groups = [list(range(g, min(g + 3, H))) for g in range(0, H, 3)]
    NG = len(groups)
    NT_ = S // 64 if nsteps is None else nsteps

    def kernel(x_hbm, mem0_ref, wq_hbm, wk_hbm, wv_hbm, wo_hbm, wr_ref, wg_hbm, wu_hbm, wd_hbm,
               out_ref,
               x_v, xn_v, r_v, st_v, w_v, wo_v, wg_v, wu_v, wd_v, fill_v,
               q_v, k_v, v_v, cq_v, o_v, co_v, acc_v,
               sem_x, sem_st, sem_wo, sem_f):
        cp_x = pltpu.make_async_copy(x_hbm, x_v, sem_x)
        cp_x.start()
        srcs = (wq_hbm, wk_hbm, wv_hbm)

        def st_copy(m, c, slot):
            return pltpu.make_async_copy(srcs[m].at[pl.ds(c * (DC * H), DC * H), :], st_v.at[slot], sem_st.at[slot])

        chunks = [(m, c) for m in range(3) for c in range(NCH)]
        for i in range(NST):
            st_copy(*chunks[i], i).start()

        cp_x.wait()
        wr = wr_ref[...].astype(F32)
        eps = float(np.asarray(1e-5, dtype=BF16).astype(np.float32))

        def ln_body(i, c):
            r0 = pl.multiple_of(i * 32, 32)
            xf = x_v[pl.ds(r0, 32), :].astype(F32)
            mean = jnp.sum(xf, axis=-1, keepdims=True) * (1.0 / D)
            cen = xf - mean
            var = jnp.sum(cen * cen, axis=-1, keepdims=True) * (1.0 / D)
            den = _rnd(jnp.sqrt(_rnd(_rnd(var) + eps)))
            xn = (_rnd(xf - _rnd(mean)) * (1.0 / den)).astype(BF16)
            for k in range(KD):
                xn_v[k, pl.ds(r0, 32), :] = xn[:, k * 128:(k + 1) * 128]
            r = _rnd(jnp.sum(xn.astype(F32) * wr, axis=-1, keepdims=True))
            r_v[pl.ds(r0, 32), :] = jnp.broadcast_to(r, (32, 128))
            return c
        jax.lax.fori_loop(0, S // 32, ln_body, 0)

        ri = jax.lax.broadcasted_iota(I32, (128, 128), 0)
        ci = jax.lax.broadcasted_iota(I32, (128, 128), 1)
        hr = (ri >= L).astype(I32) + (ri >= 2 * L).astype(I32) + (ri >= 3 * L).astype(I32)
        hc = (ci >= L).astype(I32) + (ci >= 2 * L).astype(I32) + (ci >= 3 * L).astype(I32)
        tr, tc = ri - hr * L, ci - hc * L
        vis = (tr >= SEG) | (tc >= SEG) | (tc <= tr)
        neg = float(np.asarray(-1e9, dtype=BF16).astype(np.float32))
        fill_v[...] = jnp.where(hr == hc, jnp.where(vis, 0.0, neg), -jnp.inf)

        for i, (m, c) in enumerate(chunks):
            slot = i % NST
            st_copy(m, c, slot).wait()

            def rl_body(j, carry, m=m, c=c, slot=slot):
                blk = st_v[slot, pl.ds(pl.multiple_of(j * (16 * H), 16 * H), 16 * H), :].reshape(16, H, 128)
                y = pltpu.bitcast(jnp.swapaxes(blk, 0, 1), U32)
                w_v[m, :, pl.ds(pl.multiple_of(c * (DC // 2) + j * 8, 8), 8), :] = y
                return carry
            jax.lax.fori_loop(0, DC // 16, rl_body, 0)
            if i + NST < len(chunks):
                st_copy(*chunks[i + NST], slot).start()
            if i + NST == len(chunks):
                for n in range(KD):
                    pltpu.make_async_copy(wo_hbm.at[:, pl.ds(n * 128, 128)], wo_v.at[n], sem_wo.at[n]).start()
        ffn_cps = []
        for n in range(NF):
            ffn_cps.append(pltpu.make_async_copy(wg_hbm.at[:, pl.ds(n * 128, 128)], wg_v.at[n], sem_f.at[0]))
            ffn_cps.append(pltpu.make_async_copy(wu_hbm.at[:, pl.ds(n * 128, 128)], wu_v.at[n], sem_f.at[1]))
        for n in range(KD):
            ffn_cps.append(pltpu.make_async_copy(wd_hbm.at[:, pl.ds(n * 128, 128)], wd_v.at[n], sem_f.at[2]))
        for n in range(KD):
            pltpu.make_async_copy(wo_hbm.at[:, pl.ds(n * 128, 128)], wo_v.at[n], sem_wo.at[n]).wait()
        for cp in ffn_cps:
            cp.start()

        def xrows(r0, n):
            return jnp.concatenate([xn_v[k, pl.ds(r0, n), :] for k in range(KD)], axis=1)

        def step(first, r0, mem):
            if first:
                xa = xrows(r0, 32)
                xb = xrows(r0 + 32, 16).astype(F32)[:8]
                lhs = jnp.concatenate([xa, jnp.concatenate([xb, mem], axis=0).astype(BF16)], axis=0)
            else:
                xb = xrows(r0 + 32, 16).astype(F32)[8:]
                xa = xrows(r0 + 48, 16)
                lhs = jnp.concatenate([jnp.concatenate([mem, xb], axis=0).astype(BF16), xa], axis=0)
            bufs = (q_v, k_v, v_v)
            pend = {}

            def proj(m, h):
                y = _dot(lhs, pltpu.bitcast(w_v[m, h], BF16))
                if first:
                    cq_v[m, h] = y[32:40]
                    tok = jnp.concatenate([y[:32], y[40:48]], axis=0)
                else:
                    tok = jnp.concatenate([cq_v[m, h], y[8:32], y[:8]], axis=0)
                g, j = divmod(h, 3)
                pend.setdefault((m, g), []).append(tok)
                if j == len(groups[g]) - 1:
                    toks = pend.pop((m, g))
                    n = len(toks) * L
                    pad = -n % 16
                    if pad:
                        toks.append(jnp.zeros((pad, 128), F32))
                    bufs[m][g, :n + pad, :] = jnp.concatenate(toks, axis=0).astype(BF16)

            st = {}

            def scores(g):
                n = -(-len(groups[g]) * L // 16) * 16
                s = jax.lax.dot_general(q_v[g, :n, :], k_v[g, :n, :], NT, preferred_element_type=F32)
                nv = len(groups[g]) * L
                s = s[:nv]
                fill = fill_v[:nv, :n]
                s = jnp.where(fill == 0.0, s * scale, fill)
                e = jnp.exp(s - jnp.max(s, axis=-1, keepdims=True))
                inv = 1.0 / jnp.sum(e, axis=-1, keepdims=True)
                if n > nv:
                    e = jnp.concatenate([e, jnp.zeros((n - nv, n), F32)], axis=0)
                st[g] = (e.astype(BF16), inv)

            def pv(g):
                p, inv = st.pop(g)
                n = p.shape[0]
                nv = len(groups[g]) * L
                o = _dot(p, v_v[g, :n, :])[:nv] * inv
                for j, h in enumerate(groups[g]):
                    oh = o[j * L:(j + 1) * L]
                    if first:
                        co_v[h] = oh[24:32]
                        o_v[:32, h * 128:(h + 1) * 128] = jnp.concatenate([oh[:24], oh[32:40]], axis=0).astype(BF16)
                    else:
                        o_v[:48, h * 128:(h + 1) * 128] = jnp.concatenate([co_v[h], oh], axis=0).astype(BF16)

            mo = 32 if first else 48
            acc = [None] * KD

            def wo(n, h0, h1):
                y = _dot(o_v[:mo, h0 * 128:h1 * 128], wo_v[n, h0 * 128:h1 * 128, :])
                if h0 == 0:
                    acc_v[:mo, n * 128:(n + 1) * 128] = y
                elif h1 < H:
                    acc_v[:mo, n * 128:(n + 1) * 128] += y
                else:
                    acc[n] = acc_v[:mo, n * 128:(n + 1) * 128] + y

            tasks = []
            for g in range(NG):
                pj = [(proj, m, h) for m in (1, 0, 2) for h in groups[g]]
                if g > 0:
                    a = len(pj) // 3
                    pj = pj[:a] + [(scores, g - 1)] + pj[a:] + [(pv, g - 1)]
                tasks += pj
            HS = 24
            w1 = [(wo, n, 0, HS) for n in range(KD)]
            tasks += w1[:2] + [(scores, NG - 1)] + w1[2:5] + [(pv, NG - 1)] + w1[5:]
            tasks += [(wo, n, HS, H) for n in range(KD)]
            for t in tasks:
                t[0](*t[1:])
            return jnp.concatenate(acc, axis=1)

        def base(r0, n):
            return x_v[pl.ds(r0, n), :].astype(F32) + xrows(r0, n).astype(F32)

        def macro(t, mem):
            r0 = pl.multiple_of(t * 64, 64)
            ya = step(True, r0, mem)
            out_ref[pl.ds(r0, 16), :] = (base(r0, 16) + ya[:16]).astype(BF16)
            yb = step(False, r0, ya[24:32])
            rest = jnp.concatenate([ya[16:24], yb[:40]], axis=0)
            out_ref[pl.ds(r0 + 16, 48), :] = (base(r0 + 16, 48) + rest).astype(BF16)
            return yb[40:48]

        jax.lax.fori_loop(0, NT_, macro, mem0_ref[...].astype(F32))

        rv = r_v[...]
        key = jnp.where(rv == rv, rv, -jnp.inf)
        row = jax.lax.broadcasted_iota(I32, (S, 128), 0)
        m1 = jnp.max(key, axis=0, keepdims=True)
        i1v = jnp.min(jnp.where(key == m1, row, S), axis=0, keepdims=True)
        key2 = jnp.where(row == i1v, -jnp.inf, key)
        m2 = jnp.max(key2, axis=0, keepdims=True)
        i2v = jnp.min(jnp.where((key2 == m2) & (row != i1v), row, S), axis=0, keepdims=True)
        idx = [jnp.min(i1v), jnp.min(i2v)]
        sub = jax.lax.broadcasted_iota(I32, (16, 1), 0)
        xsel = jnp.zeros((16, D), F32)
        gate = jnp.zeros((16, 1), F32)
        b0 = []
        for c in range(2):
            b = pl.multiple_of((idx[c] // 16) * 16, 16)
            b0.append(b)
            hit = sub == (idx[c] - b)
            rowv = jnp.sum(jnp.where(hit, xrows(b, 16).astype(F32), 0.0), axis=0, keepdims=True)
            rsel = jnp.sum(jnp.where(hit, r_v[pl.ds(b, 16), :][:, :1], 0.0), axis=0, keepdims=True)
            xsel = jnp.where(sub == c, rowv, xsel)
            gate = jnp.where(sub == c, _rnd(jax.nn.sigmoid(rsel)), gate)
        xsel = xsel.astype(BF16)
        for cp in ffn_cps:
            cp.wait()
        hs = []
        for n in range(NF):
            g = _rnd(_dot(xsel, wg_v[n]))
            u = _rnd(_dot(xsel, wu_v[n]))
            hs.append((_rnd(g * _rnd(jax.nn.sigmoid(g))) * u).astype(BF16))
        hid = jnp.concatenate(hs, axis=1)
        y = jnp.concatenate([_dot(hid, wd_v[n]) for n in range(KD)], axis=1)
        y = _rnd(_rnd(y) * gate)
        for c in range(2):
            hit = sub == (idx[c] - b0[c])
            blk = out_ref[pl.ds(b0[c], 16), :].astype(F32)
            out_ref[pl.ds(b0[c], 16), :] = jnp.where(hit, blk + y[c:c + 1], blk).astype(BF16)

    scratch = [
        pltpu.VMEM((S, D), BF16),
        pltpu.VMEM((KD, S, 128), BF16),
        pltpu.VMEM((S, 128), F32),
        pltpu.VMEM((NST, DC * H, 128), BF16),
        pltpu.VMEM((3, H, D // 2, 128), U32),
        pltpu.VMEM((KD, H * Dh, 128), BF16),
        pltpu.VMEM((NF, D, 128), BF16),
        pltpu.VMEM((NF, D, 128), BF16),
        pltpu.VMEM((KD, F, 128), BF16),
        pltpu.VMEM((128, 128), F32),
        pltpu.VMEM((NG, 128, 128), BF16),
        pltpu.VMEM((NG, 128, 128), BF16),
        pltpu.VMEM((NG, 128, 128), BF16),
        pltpu.VMEM((3, H, 8, 128), F32),
        pltpu.VMEM((48, H * Dh), BF16),
        pltpu.VMEM((H, 8, 128), F32),
        pltpu.VMEM((48, D), F32),
        pltpu.SemaphoreType.DMA(()),
        pltpu.SemaphoreType.DMA((NST,)),
        pltpu.SemaphoreType.DMA((KD,)),
        pltpu.SemaphoreType.DMA((3,)),
    ]
    return kernel, scratch


def run(A_x, A_mem0, A_Wq, A_Wk, A_Wv, A_Wo, A_seg_len, B_x, B_w_r, B_w_gate, B_w_up, B_w_down, **kw):
    B, S, D = A_x.shape
    _, H, Dh = A_Wq.shape
    M = A_mem0.shape[1]
    F = B_w_gate.shape[1]
    kernel, scratch = make_kernel(S, D, H, Dh, M, int(A_seg_len), F, **kw)
    hbm = pl.BlockSpec(memory_space=pl.ANY)
    vmem = pl.BlockSpec(memory_space=pltpu.VMEM)
    out = pl.pallas_call(
        kernel,
        out_shape=jax.ShapeDtypeStruct((S, D), A_x.dtype),
        in_specs=[hbm, vmem, hbm, hbm, hbm, hbm, vmem, hbm, hbm, hbm],
        out_specs=vmem,
        scratch_shapes=scratch,
        compiler_params=pltpu.CompilerParams(vmem_limit_bytes=110 * 1024 * 1024),
    )(A_x.reshape(S, D), A_mem0.reshape(M, D), A_Wq.reshape(D * H, Dh), A_Wk.reshape(D * H, Dh),
      A_Wv.reshape(D * H, Dh), A_Wo.reshape(H * Dh, D), B_w_r.reshape(1, D), B_w_gate, B_w_up, B_w_down)
    return out.reshape(B, S, D)


@functools.partial(jax.jit, static_argnames=("A_seg_len",))
def pallas_parallel_sum__memory_aug_recurrent_mem_tr__moe_arch_mod__prompt_kernel(
    A_x, A_mem0, A_Wq, A_Wk, A_Wv, A_Wo, A_seg_len, B_x, B_w_r, B_w_gate, B_w_up, B_w_down,
):
    return run(A_x, A_mem0, A_Wq, A_Wk, A_Wv, A_Wo, A_seg_len, B_x, B_w_r, B_w_gate, B_w_up, B_w_down)
```

```python
import functools
import jax
import jax.numpy as jnp
import numpy as np
import jax.experimental.pallas as pl
import jax.experimental.pallas.tpu as pltpu

F32, BF16, U32, I32 = jnp.float32, jnp.bfloat16, jnp.uint32, jnp.int32
NT = (((1,), (1,)), ((), ()))


def _rnd(v):
    return v.astype(BF16).astype(F32)


def _dot(a, b):
    return jnp.dot(a, b, preferred_element_type=F32)


def _words(v):
    return pltpu.bitcast(v, U32)


def _halves(v):
    return pltpu.bitcast(v, BF16)


def make_kernel(S, D, H, Dh, M, SEG, F, nsteps=None, MB=128, cuts=(0, 12, 27, 32), early=12, d_ps=160, d_sv=480, d_vo=300, norm_first=True, ffn=True, attn=True, split=1, onebuf=True, pin=True, lag=2):
    assert (Dh, M, SEG) == (128, 8, 32) and D % 128 == 0 and F % 128 == 0 and S % 64 == 0
    KD, NF = D // 128, F // 128
    L = M + SEG
    NSEG = S // SEG
    NMAC = S // 64
    HC = 8
    NHG = H // HC
    NPRE = NSEG * 8
    scale = Dh ** -0.5
    groups = [list(range(g, min(g + 3, H))) for g in range(0, H, 3)]
    NG = len(groups)
    NT_ = NMAC if nsteps is None else nsteps
    WR = D // 2
    WO0 = (3 * H + HC) * WR
    XN0 = WO0 + KD * H * Dh // 2
    RS0 = XN0 + KD * S // 2
    eps = float(np.asarray(1e-5, dtype=BF16).astype(np.float32))
    neg = float(np.asarray(-1e9, dtype=BF16).astype(np.float32))

    def plan(mo):
        projs = [("p", m, h) for g in groups for m in (1, 0, 2) for h in g]
        outs = [("o", n, h0, h1) for h0, h1 in zip(cuts[:-1], cuts[1:]) for n in range(KD)]
        now, done, order = 0, {}, []
        ns = nv = 0
        while projs or outs or nv < NG:
            due = []
            if nv < ns and ("p", 2, groups[nv][-1]) in done:
                due.append((max(done["s", nv] + d_sv, done["p", 2, groups[nv][-1]] + d_ps), ("v", nv)))
            if ns < NG and ("p", 0, groups[ns][-1]) in done:
                due.append((done["p", 0, groups[ns][-1]] + d_ps, ("s", ns)))
            if outs and ("v", (outs[0][3] - 1) // 3) in done and (not projs or outs[0][3] <= early):
                due.append((done["v", (outs[0][3] - 1) // 3] + d_vo, outs[0]))
            ready = [d for d in due if d[0] <= now]
            task = ready[0][1] if ready else projs[0] if projs else min(due)[1]
            if task[0] == "p":
                projs.pop(0)
                now += KD * 32 // 4
            elif task[0] == "o":
                outs.pop(0)
                now += (task[3] - task[2]) * mo // 4
            else:
                now += 32
                ns, nv = ns + (task[0] == "s"), nv + (task[0] == "v")
            done[task] = now
            order.append(task)
        return order

    def kernel(x_hbm, x3_hbm, mem0_ref, wq_hbm, wk_hbm, wv_hbm, wo_hbm, wr_ref, wg_hbm, wu_hbm, wd_hbm,
               out_hbm,
               x_v, xp_v, xpre_v, st_v, w_v, wost_v, pre_v, wg_v, wu_v, wd_v, y_v,
               fill_v, q_v, k_v, v_v, o_v, co_v, acc_v, out_v, tab_s,
               sem_xp, sem_x, sem_st, sem_wo, sem_f, sem_out, sem_fix):
        srcs = (wq_hbm, wk_hbm, wv_hbm)
        WOFF = (2 * H, 0, H)
        XR = S // NHG

        def st_copy(m, hg):
            return pltpu.make_async_copy(
                srcs[m].at[:, pl.ds(pl.multiple_of(hg * HC, HC), HC), :], st_v.at[m], sem_st.at[m])

        def x_copy(hg):
            rows = pl.ds(pl.multiple_of(hg * XR, XR), XR)
            return pltpu.make_async_copy(x_hbm.at[rows, :], x_v.at[rows, :], sem_x)

        def wo_copy(hg, j):
            cols = pl.ds(pl.multiple_of((hg * (KD // NHG) + j) * 128, 128), 128)
            return pltpu.make_async_copy(wo_hbm.at[:, cols], wost_v.at[j], sem_wo.at[j])

        def ffn_copies(j, slot):
            f0 = pl.ds(pl.multiple_of(j * 128, 128), 128)
            return (pltpu.make_async_copy(wg_hbm.at[:, f0], wg_v.at[slot], sem_f.at[3 * slot]),
                    pltpu.make_async_copy(wu_hbm.at[:, f0], wu_v.at[slot], sem_f.at[3 * slot + 1]),
                    pltpu.make_async_copy(wd_hbm.at[f0, :], wd_v.at[slot], sem_f.at[3 * slot + 2]))

        def out_copy(t):
            rows = pl.ds(pl.multiple_of(t * 64, 64), 64)
            return pltpu.make_async_copy(out_v.at[rows, :], out_hbm.at[rows, :], sem_out)

        def layernorm(xf):
            mean = jnp.sum(xf, axis=-1, keepdims=True) * (1.0 / D)
            cen = xf - mean
            var = jnp.sum(cen * cen, axis=-1, keepdims=True) * (1.0 / D)
            den = _rnd(jnp.sqrt(_rnd(_rnd(var) + eps)))
            return (_rnd(xf - _rnd(mean)) * (1.0 / den)).astype(BF16)

        def rows(start, n):
            return pl.ds(start if isinstance(start, int) else pl.multiple_of(start, 8), n)

        def weight(m, h):
            return _halves(w_v[rows((WOFF[m] + h) * WR, WR), :])

        def normed(r0, n):
            return _halves(jnp.concatenate([w_v[rows(XN0 + k * (S // 2) + r0 // 2, n // 2), :] for k in range(KD)], axis=1))

        def relayout(m, h0):
            def piece(d0):
                y = _words(jnp.swapaxes(st_v[m, pl.ds(d0, 16)], 0, 1))
                for hh in range(HC):
                    w_v[rows((WOFF[m] + h0 + hh) * WR + d0 // 2, 8), :] = y[hh]
            return [functools.partial(piece, d0) for d0 in range(0, D, 16)]

        def weave(*jobs):
            order = sorted(((i + 0.5) / len(js), n, i) for n, js in enumerate(jobs) for i in range(len(js)))
            for _, n, i in order:
                jobs[n][i]()

        cp_xp = pltpu.make_async_copy(x3_hbm.at[:, pl.ds(0, 8), :], xp_v, sem_xp)
        cp_xp.start()
        st_copy(0, 0).start()

        ri = jax.lax.broadcasted_iota(I32, (128, 128), 0)
        ci = jax.lax.broadcasted_iota(I32, (128, 128), 1)
        hr = (ri >= L).astype(I32) + (ri >= 2 * L).astype(I32) + (ri >= 3 * L).astype(I32)
        hc = (ci >= L).astype(I32) + (ci >= 2 * L).astype(I32) + (ci >= 3 * L).astype(I32)
        tr, tc = ri - hr * L, ci - hc * L
        vis = (tr >= SEG) | (tc >= SEG) | (tc <= tr)
        fill_v[...] = jnp.where(hr == hc, jnp.where(vis, 0.0, neg), -jnp.inf)
        y_v[...] = jnp.zeros(y_v.shape, F32)
        for i in range(NHG):
            tab_s[i] = i

        cp_xp.wait()
        st_copy(1, 0).start()

        def pre_ln(i, c):
            xf = jnp.concatenate([xp_v[i * 8 + j].astype(F32) for j in range(8)], axis=0)
            w = _words(layernorm(xf))
            for k in range(KD):
                xpre_v[k, pl.ds(pl.multiple_of(i * 32, 32), 32), :] = w[:, k * 128:(k + 1) * 128]
            return c
        jax.lax.fori_loop(0, NSEG // 8, pre_ln, 0)

        st_copy(0, 0).wait()
        x_copy(0).start()
        st_copy(2, 0).start()
        weave(relayout(0, 0))

        wr = wr_ref[...].astype(F32)

        lane = jax.lax.broadcasted_iota(I32, (16, 128), 1)
        sub = jax.lax.broadcasted_iota(I32, (16, 1), 0)

        def project_pre(m, h0, zero=None):
            def piece(hh, r):
                lhs = _halves(jnp.concatenate([xpre_v[k, r // 2:(r + MB) // 2, :] for k in range(KD)], axis=1))
                y = _dot(lhs, weight(m, h0 + hh)).astype(BF16)
                pre_v[m, h0 + hh, r // 2:(r + MB) // 2, :] = _words(y)
                if zero is not None:
                    x_v[pl.ds(pl.multiple_of(S + zero, 16), 16), :128] = y[:16]
            return [functools.partial(piece, hh, r) for hh in range(HC) for r in range(0, NPRE, MB)]

        def norm_rows(r0, half0, n, score):
            held = {}

            def compute(r):
                xn = layernorm(x_v[pl.ds(pl.multiple_of(r0 + r, 16), 16), :].astype(F32))
                held[r] = _words(xn), _rnd(jnp.sum(xn.astype(F32) * wr, axis=-1, keepdims=True))

            def commit(r):
                xw, sc = held.pop(r)
                for k in range(KD):
                    w_v[rows(XN0 + k * (S // 2) + half0 + r // 2, 8), :] = xw[:, k * 128:(k + 1) * 128]
                score[0] = jnp.where(lane == (r0 + r) // 16, sc, score[0])
                w_v[rows(RS0 + half0 - half0 // 8 * 8, 16), :] = pltpu.bitcast(score[0], U32)

            rs = list(range(0, n, 16))
            nop = [lambda: None] * lag
            return ([functools.partial(compute, r) for r in rs] + nop, nop + [functools.partial(commit, r) for r in rs])

        def repack_wo(hg):
            def piece(j, r):
                w_v[rows(WO0 + (hg * (KD // NHG) + j) * (H * Dh // 2) + r // 2, 128), :] = _words(wost_v[j, r:r + 256, :])
            return [functools.partial(piece, j, r) for j in range(KD // NHG) for r in range(0, H * Dh, 256)]

        def pre_body(hg, score):
            h0 = pl.multiple_of(hg * HC, HC)
            more = hg + 1 < NHG
            sg = tab_s[hg] if pin else hg
            zero = tab_s[0]
            score = [score]

            @pl.when(more)
            def _():
                st_copy(0, hg + 1).start()
                for j in range(KD // NHG):
                    wo_copy(hg, j).start()
            st_copy(1, hg).wait()
            weave(project_pre(0, h0), relayout(1, sg * HC))

            @pl.when(more)
            def _():
                st_copy(1, hg + 1).start()
            st_copy(2, hg).wait()
            x_copy(hg).wait()
            weave(project_pre(1, h0, zero), relayout(2, sg * HC), *norm_rows(hg * XR, sg * (XR // 2), XR // 2, score))

            @pl.when(more)
            def _():
                st_copy(2, hg + 1).start()
                x_copy(hg + 1).start()
                st_copy(0, hg + 1).wait()
            for j in range(KD // NHG):
                wo_copy(hg, j).wait()
            weave(project_pre(2, h0, zero), relayout(0, sg * HC + HC),
                  *norm_rows(hg * XR + XR // 2, sg * (XR // 2) + XR // 4, XR // 2, score), repack_wo(sg))

            @pl.when(hg + 2 == NHG)
            def _():
                for j in range(KD // NHG):
                    wo_copy(hg + 1, j).start()
            return score[0]

        for cp in ffn_copies(0, 0) + ffn_copies(1, 1):
            cp.start()
        score = jax.lax.fori_loop(0, NHG, pre_body, jnp.zeros((16, 128), F32))

        def first_max(key, free):
            top = jnp.max(jnp.max(key, axis=1, keepdims=True), axis=0, keepdims=True)
            return top, jnp.min(jnp.where((key == top) & free, tok_id, S))

        tok_id = lane * 16 + sub
        key = jnp.where(score == score, score, -jnp.inf)
        m1, i1 = first_max(key, tok_id >= 0)
        m2, i2 = first_max(jnp.where(tok_id == i1, -jnp.inf, key), tok_id != i1)
        idx = [i1, i2]
        gate = jnp.where(sub == 0, _rnd(jax.nn.sigmoid(m1)), _rnd(jax.nn.sigmoid(m2)))
        xsel = jnp.zeros((16, D), F32)
        blk0 = []
        for c in range(2):
            b = pl.multiple_of((idx[c] // 16) * 16, 16)
            blk0.append(b)
            rowv = jnp.sum(jnp.where(sub == idx[c] - b, normed(b, 16).astype(F32), 0.0), axis=0, keepdims=True)
            xsel = jnp.where(sub == c, rowv, xsel)
        xsel = xsel.astype(BF16)

        def step(first, t, mem, filler):
            r0 = pl.multiple_of(t * 64 + (0 if first else 32), 32)
            xs = normed(r0, 32)
            lhs = jnp.concatenate(
                [jnp.concatenate([mem, xs[:16].astype(F32)[8:]], axis=0).astype(BF16), xs[16:]], axis=0)
            bufs = (q_v, k_v, v_v)
            pend = {}

            def proj(m, h):
                y = _dot(lhs, weight(m, h))
                pre = _halves(pre_v[m, h, pl.ds(pl.multiple_of(t * 8, 8), 8), :]).astype(F32)
                tok = jnp.concatenate([pre[:8] if first else pre[8:], y[8:], y[:8]], axis=0)
                g, j = divmod(h, 3)
                pend.setdefault((m, g), []).append(tok)
                if j == len(groups[g]) - 1:
                    toks = pend.pop((m, g))
                    n = len(toks) * L
                    pad = -n % 16
                    if pad:
                        toks.append(jnp.zeros((pad, 128), F32))
                    bufs[m][g, :(n + pad) // 2, :] = _words(jnp.concatenate(toks, axis=0).astype(BF16))

            st = {}

            def scores(g):
                nv = len(groups[g]) * L
                n = -(-nv // 16) * 16
                if not attn:
                    return
                rb = n if split == 1 else 128 // split
                kk = _halves(k_v[g, :n // 2, :])
                s = jnp.concatenate([jax.lax.dot_general(_halves(q_v[g, r // 2:min(r + rb, n) // 2, :]), kk, NT,
                                                         preferred_element_type=F32) for r in range(0, n, rb)], axis=0)[:nv]
                fill = fill_v[:nv, :n]
                s = jnp.where(fill == 0.0, s * scale, fill)
                e = jnp.exp(s - jnp.max(s, axis=-1, keepdims=True))
                inv = 1.0 / jnp.sum(e, axis=-1, keepdims=True)
                if norm_first:
                    e, inv = e * inv, None
                if n > nv:
                    e = jnp.concatenate([e, jnp.zeros((n - nv, n), F32)], axis=0)
                st[g] = (e.astype(BF16), inv)

            def pv(g):
                nv = len(groups[g]) * L
                n = -(-nv // 16) * 16
                if attn:
                    p, inv = st.pop(g)
                    rb = n if split == 1 else 128 // split
                    vv = _halves(v_v[g, :n // 2, :])
                    o = jnp.concatenate([_dot(p[r:r + rb], vv) for r in range(0, n, rb)], axis=0)[:nv]
                else:
                    inv = None
                    o = (_halves(v_v[g, :n // 2, :]).astype(F32) + _halves(k_v[g, :n // 2, :]).astype(F32) + _halves(q_v[g, :n // 2, :]).astype(F32))[:nv] * 0.01
                if inv is not None:
                    o = o * inv
                for j, h in enumerate(groups[g]):
                    oh = o[j * L:(j + 1) * L]
                    if first:
                        co_v[h] = oh[24:32]
                        o_v[h, :16, :] = _words(jnp.concatenate([oh[:24], oh[32:40]], axis=0).astype(BF16))
                    else:
                        o_v[h, :24, :] = _words(jnp.concatenate([co_v[h], oh], axis=0).astype(BF16))

            mo = 32 if first else 48
            acc = [None] * KD

            def wo(n, h0, h1):
                lhs_o = _halves(jnp.concatenate([o_v[h, :mo // 2, :] for h in range(h0, h1)], axis=1))
                y = _dot(lhs_o, _halves(w_v[rows(WO0 + n * (H * Dh // 2) + h0 * 64, (h1 - h0) * 64), :]))
                if h0 == 0:
                    acc_v[:mo, n * 128:(n + 1) * 128] = y
                elif h1 < H:
                    acc_v[:mo, n * 128:(n + 1) * 128] += y
                else:
                    acc[n] = acc_v[:mo, n * 128:(n + 1) * 128] + y

            tasks = [({"p": proj, "s": scores, "v": pv, "o": wo}[tk[0]],) + tk[1:] for tk in plan(mo)]
            for tk in tasks:
                tk[0](*tk[1:])
            filler()
            return jnp.concatenate(acc, axis=1)

        def base(r0, n):
            return x_v[pl.ds(r0, n), :].astype(F32) + normed(r0, n).astype(F32)

        def macro(t, mem):
            r0 = pl.multiple_of(t * 64, 64)
            slot = t % 2
            for cp in ffn_copies(jnp.minimum(t, NF - 1), slot):
                cp.wait()
            hid = []

            def ffn_up():
                if ffn:
                    g = _rnd(_dot(xsel, wg_v[slot]))
                    u = _rnd(_dot(xsel, wu_v[slot]))
                    hid.append(jnp.where(t < NF, _rnd(g * _rnd(jax.nn.sigmoid(g))) * u, 0.0).astype(BF16))

            def ffn_down():
                if ffn:
                    y_v[...] += _dot(hid[0], wd_v[slot])

            ya = step(True, t, mem, ffn_up)
            out_v[pl.ds(r0, 16), :] = (base(r0, 16) + ya[:16]).astype(BF16)
            yb = step(False, t, ya[24:32], ffn_down)
            rest = jnp.concatenate([ya[16:24], yb[:40]], axis=0)
            out_v[pl.ds(r0 + 16, 48), :] = (base(r0 + 16, 48) + rest).astype(BF16)
            out_copy(t).start()
            for cp in ffn_copies(jnp.minimum(t + 2, NF - 1), slot):
                cp.start()
            return yb[40:48]

        jax.lax.fori_loop(0, NT_, macro, mem0_ref[...].astype(F32))

        for cp in ffn_copies(NF - 1, 0) + ffn_copies(NF - 1, 1):
            cp.wait()
        done = pl.ds(0, NT_ * 64)
        pltpu.make_async_copy(out_v.at[done, :], out_hbm.at[done, :], sem_out).wait()

        y = _rnd(_rnd(y_v[...]) * gate)
        for c in range(2):
            blk = out_v[pl.ds(blk0[c], 16), :].astype(F32)
            out_v[pl.ds(blk0[c], 16), :] = jnp.where(sub == idx[c] - blk0[c], blk + y[c:c + 1], blk).astype(BF16)
        fix = [pltpu.make_async_copy(out_v.at[pl.ds(blk0[c], 16), :], out_hbm.at[pl.ds(blk0[c], 16), :], sem_fix.at[c])
               for c in range(2)]
        fix[0].start()

        @pl.when(blk0[0] != blk0[1])
        def _():
            fix[1].start()
            fix[1].wait()
        fix[0].wait()

    scratch = [
        pltpu.VMEM((S + 16, D), BF16),
        pltpu.VMEM((NSEG, 8, D), BF16),
        pltpu.VMEM((KD, NPRE // 2, 128), U32),
        pltpu.VMEM((3, D, HC, 128), BF16),
        pltpu.VMEM((RS0 + 16, 128), U32),
        pltpu.VMEM((KD // NHG, H * Dh, 128), BF16),
        pltpu.VMEM((3, H, NPRE // 2, 128), U32),
        pltpu.VMEM((2, D, 128), BF16),
        pltpu.VMEM((2, D, 128), BF16),
        pltpu.VMEM((2, 128, D), BF16),
        pltpu.VMEM((16, D), F32),
        pltpu.VMEM((128, 128), F32),
        pltpu.VMEM((NG, 64, 128), U32),
        pltpu.VMEM((NG, 64, 128), U32),
        pltpu.VMEM((NG, 64, 128), U32),
        pltpu.VMEM((H, 24, 128), U32),
        pltpu.VMEM((H, 8, 128), F32),
        pltpu.VMEM((48, D), F32),
        pltpu.VMEM((S, D), BF16),
        pltpu.SMEM((NHG,), I32),
        pltpu.SemaphoreType.DMA(()),
        pltpu.SemaphoreType.DMA(()),
        pltpu.SemaphoreType.DMA((3,)),
        pltpu.SemaphoreType.DMA((KD // NHG,)),
        pltpu.SemaphoreType.DMA((6,)),
        pltpu.SemaphoreType.DMA(()),
        pltpu.SemaphoreType.DMA((2,)),
    ]
    return kernel, scratch


def run(A_x, A_mem0, A_Wq, A_Wk, A_Wv, A_Wo, A_seg_len, B_x, B_w_r, B_w_gate, B_w_up, B_w_down, **kw):
    B, S, D = A_x.shape
    _, H, Dh = A_Wq.shape
    M = A_mem0.shape[1]
    F = B_w_gate.shape[1]
    seg = int(A_seg_len)
    kernel, scratch = make_kernel(S, D, H, Dh, M, seg, F, **kw)
    hbm = pl.BlockSpec(memory_space=pl.ANY)
    vmem = pl.BlockSpec(memory_space=pltpu.VMEM)
    out = pl.pallas_call(
        kernel,
        out_shape=jax.ShapeDtypeStruct((S, D), A_x.dtype),
        in_specs=[hbm, hbm, vmem, hbm, hbm, hbm, hbm, vmem, hbm, hbm, hbm],
        out_specs=hbm,
        scratch_shapes=scratch,
        compiler_params=pltpu.CompilerParams(vmem_limit_bytes=110 * 1024 * 1024),
    )(A_x.reshape(S, D), A_x.reshape(S // seg, seg, D), A_mem0.reshape(M, D), A_Wq, A_Wk, A_Wv,
      A_Wo.reshape(H * Dh, D), B_w_r.reshape(1, D), B_w_gate, B_w_up, B_w_down)
    return out.reshape(B, S, D)


@functools.partial(jax.jit, static_argnames=("A_seg_len",))
def pallas_parallel_sum__memory_aug_recurrent_mem_tr__moe_arch_mod__prompt_kernel(
    A_x, A_mem0, A_Wq, A_Wk, A_Wv, A_Wo, A_seg_len, B_x, B_w_r, B_w_gate, B_w_up, B_w_down,
):
    return run(A_x, A_mem0, A_Wq, A_Wk, A_Wv, A_Wo, A_seg_len, B_x, B_w_r, B_w_gate, B_w_up, B_w_down)
```

```python
import functools
import jax
import jax.numpy as jnp
import numpy as np
import jax.experimental.pallas as pl
import jax.experimental.pallas.tpu as pltpu

F32, BF16, U32, I32 = jnp.float32, jnp.bfloat16, jnp.uint32, jnp.int32
NT = (((1,), (1,)), ((), ()))


def _rnd(v):
    return v.astype(BF16).astype(F32)


def _dot(a, b):
    return jnp.dot(a, b, preferred_element_type=F32)


def _words(v):
    return pltpu.bitcast(v, U32)


def _halves(v):
    return pltpu.bitcast(v, BF16)


def make_kernel(S, D, H, Dh, M, SEG, F, nsteps=None, MB=64, cuts=(0, 12, 27, 32), early=12, d_ps=160, d_sv=480, d_vo=300, norm_first=True, ffn=True, attn=True, split=1, onebuf=True, pin=True, lag=1, ln_cut=272, dn_at=None, staged=True, up_rows=32, dn_rows=16):
    assert (Dh, M, SEG) == (128, 8, 32) and D % 128 == 0 and F % 128 == 0 and S % 64 == 0
    KD, NF = D // 128, F // 128
    L = M + SEG
    NSEG = S // SEG
    NMAC = S // 64
    HC = 8
    NHG = H // HC
    OR = 512
    NWO = -(-(H * Dh // OR) // (NHG - 1))
    NPRE = NSEG * 8
    scale = Dh ** -0.5
    groups = [list(range(g, min(g + 3, H))) for g in range(0, H, 3)]
    NG = len(groups)
    NT_ = NMAC if nsteps is None else nsteps
    WR = D // 2
    WO0 = (3 * H + HC) * WR
    XN0 = WO0 + KD * H * Dh // 2
    RS0 = XN0 + KD * S // 2
    eps = float(np.asarray(1e-5, dtype=BF16).astype(np.float32))
    neg = float(np.asarray(-1e9, dtype=BF16).astype(np.float32))

    def plan(mo):
        projs = [("p", m, h) for g in groups for m in (1, 0, 2) for h in g]
        outs = [("o", n, h0, h1) for h0, h1 in zip(cuts[:-1], cuts[1:]) for n in range(KD)]
        now, done, order = 0, {}, []
        ns = nv = 0
        while projs or outs or nv < NG:
            due = []
            if nv < ns and ("p", 2, groups[nv][-1]) in done:
                due.append((max(done["s", nv] + d_sv, done["p", 2, groups[nv][-1]] + d_ps), ("v", nv)))
            if ns < NG and ("p", 0, groups[ns][-1]) in done:
                due.append((done["p", 0, groups[ns][-1]] + d_ps, ("s", ns)))
            if outs and ("v", (outs[0][3] - 1) // 3) in done and (not projs or outs[0][3] <= early):
                due.append((done["v", (outs[0][3] - 1) // 3] + d_vo, outs[0]))
            ready = [d for d in due if d[0] <= now]
            task = ready[0][1] if ready else projs[0] if projs else min(due)[1]
            if task[0] == "p":
                projs.pop(0)
                now += KD * 32 // 4
            elif task[0] == "o":
                outs.pop(0)
                now += (task[3] - task[2]) * mo // 4
            else:
                now += 32
                ns, nv = ns + (task[0] == "s"), nv + (task[0] == "v")
            done[task] = now
            order.append(task)
        return order

    def kernel(x_hbm, x3_hbm, mem0_hbm, wq_hbm, wk_hbm, wv_hbm, wo_hbm, wr_hbm, wg_hbm, wu_hbm, wd_hbm,
               out_hbm,
               mem0_v, wr_v, x_v, xp_v, xpre_v, st_v, w_v, wost_v, pre_v, wg_v, wu_v, wd_v, y_v,
               fill_v, q_v, k_v, v_v, o_v, co_v, acc_v, out_v, tab_s,
               sem_in, sem_xp, sem_q0, sem_x, sem_st, sem_wo, sem_f, sem_out, sem_fix):
        srcs = (wq_hbm, wk_hbm, wv_hbm)
        WOFF = (2 * H, 0, H)
        XR = S // NHG

        def st_copy(m, hg, zero=0):
            return pltpu.make_async_copy(
                srcs[m].at[:, pl.ds(pl.multiple_of(hg * HC, HC), HC), :], st_v.at[m + zero], sem_st.at[m])

        def x_copy(hg, part):
            a, b = ((0, ln_cut), (ln_cut, XR))[part]
            rows = pl.ds(pl.multiple_of(hg * XR + a, 16), b - a)
            return pltpu.make_async_copy(x_hbm.at[rows, :], x_v.at[rows, :], sem_x.at[part])

        def wo_block(hg, j):
            return jnp.minimum(hg * NWO + j, H * Dh // OR - 1)

        def wo_copy(hg, j):
            rows = pl.ds(pl.multiple_of(wo_block(hg, j) * OR, OR), OR)
            return pltpu.make_async_copy(wo_hbm.at[rows, :], wost_v.at[j], sem_wo.at[j])

        def ffn_copies(j, slot):
            f0 = pl.ds(pl.multiple_of(j * 128, 128), 128)
            return (pltpu.make_async_copy(wg_hbm.at[:, f0], wg_v.at[slot], sem_f.at[3 * slot]),
                    pltpu.make_async_copy(wu_hbm.at[:, f0], wu_v.at[slot], sem_f.at[3 * slot + 1]),
                    pltpu.make_async_copy(wd_hbm.at[f0, :], wd_v.at[slot], sem_f.at[3 * slot + 2]))

        def out_copy(t):
            rows = pl.ds(pl.multiple_of(t * 64, 64), 64)
            last = jnp.where(t == NT_ - 1, 1, 0)
            return pltpu.make_async_copy(out_v.at[rows, :], out_hbm.at[rows, :], sem_out.at[last])

        def layernorm(xf):
            mean = jnp.sum(xf, axis=-1, keepdims=True) * (1.0 / D)
            cen = xf - mean
            var = jnp.sum(cen * cen, axis=-1, keepdims=True) * (1.0 / D)
            den = _rnd(jnp.sqrt(_rnd(_rnd(var) + eps)))
            return (_rnd(xf - _rnd(mean)) * (1.0 / den)).astype(BF16)

        def rows(start, n):
            return pl.ds(start if isinstance(start, int) else pl.multiple_of(start, 8), n)

        def weight(m, h):
            return _halves(w_v[rows((WOFF[m] + h) * WR, WR), :])

        def normed(r0, n):
            return _halves(jnp.concatenate([w_v[rows(XN0 + k * (S // 2) + r0 // 2, n // 2), :] for k in range(KD)], axis=1))

        def relayout(m, h0):
            def piece(d0):
                y = _words(jnp.swapaxes(st_v[m, pl.ds(d0, 16)], 0, 1))
                for hh in range(HC):
                    w_v[rows((WOFF[m] + h0 + hh) * WR + d0 // 2, 8), :] = y[hh]
            return [functools.partial(piece, d0) for d0 in range(0, D, 16)]

        def weave(*jobs):
            order = sorted(((i + 0.5) / len(js), n, i) for n, js in enumerate(jobs) for i in range(len(js)))
            for _, n, i in order:
                jobs[n][i]()

        xp_cps = [pltpu.make_async_copy(x3_hbm.at[pl.ds(i * (NSEG // 4), NSEG // 4), pl.ds(0, 8), :],
                                        xp_v.at[pl.ds(i * (NSEG // 4), NSEG // 4)], sem_xp.at[i]) for i in range(4)]
        q0_cps = [pltpu.make_async_copy(wq_hbm.at[pl.ds(i * (D // 4), D // 4), pl.ds(0, HC), :],
                                        st_v.at[0, pl.ds(i * (D // 4), D // 4)], sem_q0.at[i]) for i in range(4)]
        in_cps = [pltpu.make_async_copy(wr_hbm, wr_v, sem_in.at[0]), pltpu.make_async_copy(mem0_hbm, mem0_v, sem_in.at[1])]
        for cp in xp_cps[:2] + in_cps:
            cp.start()

        ri = jax.lax.broadcasted_iota(I32, (128, 128), 0)
        ci = jax.lax.broadcasted_iota(I32, (128, 128), 1)
        hr = (ri >= L).astype(I32) + (ri >= 2 * L).astype(I32) + (ri >= 3 * L).astype(I32)
        hc = (ci >= L).astype(I32) + (ci >= 2 * L).astype(I32) + (ci >= 3 * L).astype(I32)
        tr, tc = ri - hr * L, ci - hc * L
        vis = (tr >= SEG) | (tc >= SEG) | (tc <= tr)
        fill_v[...] = jnp.where(hr == hc, jnp.where(vis, 0.0, neg), -jnp.inf)
        y_v[...] = jnp.zeros(y_v.shape, F32)
        for i in range(NHG):
            tab_s[i] = i

        def pre_ln(i, c):
            xf = jnp.concatenate([xp_v[i * 8 + j].astype(F32) for j in range(8)], axis=0)
            w = _words(layernorm(xf))
            for k in range(KD):
                xpre_v[k, pl.ds(pl.multiple_of(i * 32, 32), 32), :] = w[:, k * 128:(k + 1) * 128]
            return c
        ahead = [xp_cps[2:] + q0_cps[:1], [], q0_cps[1:2], q0_cps[2:3], q0_cps[3:], [], [st_copy(1, 0)], []]
        for i, cp in enumerate(xp_cps):
            cp.wait()
            for nxt in ahead[i]:
                nxt.start()
            jax.lax.fori_loop(i * (NSEG // 32), (i + 1) * (NSEG // 32), pre_ln, 0)
        first_q = relayout(0, 0)
        for i, cp in enumerate(q0_cps):
            cp.wait()
            for nxt in ahead[4 + i]:
                nxt.start()
            weave(first_q[i * (len(first_q) // 4):(i + 1) * (len(first_q) // 4)])


        lane = jax.lax.broadcasted_iota(I32, (16, 128), 1)
        sub = jax.lax.broadcasted_iota(I32, (16, 1), 0)

        def project_pre(m, h0, zero=None):
            def piece(hh, r):
                lhs = _halves(jnp.concatenate([xpre_v[k, r // 2:(r + MB) // 2, :] for k in range(KD)], axis=1))
                y = _dot(lhs, weight(m, h0 + hh)).astype(BF16)
                pre_v[m, h0 + hh, r // 2:(r + MB) // 2, :] = _words(y)
                if zero is not None:
                    x_v[pl.ds(pl.multiple_of(S + zero, 16), 16), :128] = y[:16]
            return [functools.partial(piece, hh, r) for hh in range(HC) for r in range(0, NPRE, MB)]

        def norm_rows(r0, half0, n, score):
            held = {}

            def load(r):
                return x_v[pl.ds(pl.multiple_of(r0 + r, 16), 16), :].astype(F32)

            def mean(r):
                held[r] = jnp.sum(load(r), axis=-1, keepdims=True) * (1.0 / D)

            def spread(r):
                cen = load(r) - held[r]
                var = jnp.sum(cen * cen, axis=-1, keepdims=True) * (1.0 / D)
                held[r] = _rnd(held[r]), 1.0 / _rnd(jnp.sqrt(_rnd(_rnd(var) + eps)))

            def apply(r):
                mu, inv = held[r]
                xn = (_rnd(load(r) - mu) * inv).astype(BF16)
                held[r] = _words(xn), _rnd(jnp.sum(xn.astype(F32) * wr, axis=-1, keepdims=True))

            def whole(r):
                xn = layernorm(load(r))
                held[r] = _words(xn), _rnd(jnp.sum(xn.astype(F32) * wr, axis=-1, keepdims=True))

            def commit(r):
                xw = held[r][0]
                for k in range(KD):
                    w_v[rows(XN0 + k * (S // 2) + half0 + r // 2, 8), :] = xw[:, k * 128:(k + 1) * 128]

            def note(r):
                score[0] = jnp.where(lane == (r0 + r) // 16, held.pop(r)[1], score[0])
                w_v[rows(RS0 + half0 - half0 // 8 * 8, 16), :] = pltpu.bitcast(score[0], U32)

            rs = list(range(0, n, 16))
            stages = [(mean, 0), (spread, 1), (apply, 2), (commit, 2 + lag), (note, 3)] if staged else [(whole, 0), (commit, lag), (note, lag)]
            depth = max(d for _, d in stages)
            nop = [lambda: None]
            return [nop * d + [functools.partial(f, r) for r in rs] + nop * (depth - d) for f, d in stages]

        def repack_wo(hg):
            def piece(j, r):
                w = _words(wost_v[j, r:r + 32, :])
                for n in range(KD):
                    w_v[rows(WO0 + n * (H * Dh // 2) + wo_block(hg, j) * (OR // 2) + r // 2, 16), :] = w[:, n * 128:(n + 1) * 128]
            return [functools.partial(piece, j, r) for j in range(NWO) for r in range(0, OR, 32)]

        dots = project_pre(0, 0)
        weave(dots[:len(dots) // 2])
        st_copy(1, 0).wait()

        @pl.when(tab_s[0] == 0)
        def _():
            st_copy(2, 0).start()
            x_copy(0, 0).start()
        weave(dots[len(dots) // 2:], relayout(1, tab_s[0]))
        for cp in in_cps:
            cp.wait()
        wr = wr_v[...].astype(F32).reshape(1, D)

        def pre_body(hg, score):
            h0 = pl.multiple_of(hg * HC, HC)
            more = hg + 1 < NHG
            sg = tab_s[hg]
            zero = tab_s[0]
            score = [score]

            def norm(a, b):
                return norm_rows(hg * XR + a, sg * (XR // 2) + a // 2, b - a, score)

            @pl.when(more)
            def _():
                st_copy(0, hg + 1).start()
                wo_copy(hg, 0).start()

            @pl.when(jnp.logical_not(more))
            def _():
                for cp in ffn_copies(0, 0) + ffn_copies(1, 1):
                    cp.start()
            x_copy(hg, 1).start()
            st_copy(2, hg).wait()
            x_copy(hg, 0).wait()
            weave(project_pre(1, h0, zero), relayout(2, sg * HC), *norm(0, ln_cut))

            @pl.when(more)
            def _():
                st_copy(1, hg + 1).start()
                for j in range(1, NWO):
                    wo_copy(hg, j).start()
                st_copy(0, hg + 1).wait()
            x_copy(hg, 1).wait()
            weave(project_pre(2, h0, zero), relayout(0, sg * HC + HC), *norm(ln_cut, XR))

            @pl.when(more)
            def _():
                st_copy(2, hg + 1).start()
                x_copy(hg + 1, 0).start()
                st_copy(1, hg + 1).wait()
                for j in range(NWO):
                    wo_copy(hg, j).wait()
                weave(project_pre(0, h0 + HC), relayout(1, sg * HC + HC), repack_wo(sg))
            return score[0]

        score = jax.lax.fori_loop(0, NHG, pre_body, jnp.zeros((16, 128), F32))

        def first_max(key, free):
            top = jnp.max(jnp.max(key, axis=1, keepdims=True), axis=0, keepdims=True)
            return top, jnp.min(jnp.where((key == top) & free, tok_id, S))

        tok_id = lane * 16 + sub
        key = jnp.where(score == score, score, -jnp.inf)
        m1, i1 = first_max(key, tok_id >= 0)
        m2, i2 = first_max(jnp.where(tok_id == i1, -jnp.inf, key), tok_id != i1)
        idx = [i1, i2]
        gate = jnp.where(sub == 0, _rnd(jax.nn.sigmoid(m1)), _rnd(jax.nn.sigmoid(m2)))
        xsel = jnp.zeros((16, D), F32)
        blk0 = []
        for c in range(2):
            b = pl.multiple_of((idx[c] // 16) * 16, 16)
            blk0.append(b)
            rowv = jnp.sum(jnp.where(sub == idx[c] - b, normed(b, 16).astype(F32), 0.0), axis=0, keepdims=True)
            xsel = jnp.where(sub == c, rowv, xsel)
        xsel = jnp.concatenate([xsel] * (up_rows // 16), axis=0).astype(BF16)

        def step(first, t, mem, filler):
            r0 = pl.multiple_of(t * 64 + (0 if first else 32), 32)
            xs = normed(r0, 32)
            lhs = jnp.concatenate(
                [jnp.concatenate([mem, xs[:16].astype(F32)[8:]], axis=0).astype(BF16), xs[16:]], axis=0)
            bufs = (q_v, k_v, v_v)
            pend = {}

            def proj(m, h):
                y = _dot(lhs, weight(m, h))
                pre = _halves(pre_v[m, h, pl.ds(pl.multiple_of(t * 8, 8), 8), :]).astype(F32)
                tok = jnp.concatenate([pre[:8] if first else pre[8:], y[8:], y[:8]], axis=0)
                g, j = divmod(h, 3)
                pend.setdefault((m, g), []).append(tok)
                if j == len(groups[g]) - 1:
                    toks = pend.pop((m, g))
                    n = len(toks) * L
                    pad = -n % 16
                    if pad:
                        toks.append(jnp.zeros((pad, 128), F32))
                    bufs[m][g, :(n + pad) // 2, :] = _words(jnp.concatenate(toks, axis=0).astype(BF16))

            st = {}

            def scores(g):
                nv = len(groups[g]) * L
                n = -(-nv // 16) * 16
                if not attn:
                    return
                rb = n if split == 1 else 128 // split
                kk = _halves(k_v[g, :n // 2, :])
                s = jnp.concatenate([jax.lax.dot_general(_halves(q_v[g, r // 2:min(r + rb, n) // 2, :]), kk, NT,
                                                         preferred_element_type=F32) for r in range(0, n, rb)], axis=0)[:nv]
                fill = fill_v[:nv, :n]
                s = jnp.where(fill == 0.0, s * scale, fill)
                e = jnp.exp(s - jnp.max(s, axis=-1, keepdims=True))
                inv = 1.0 / jnp.sum(e, axis=-1, keepdims=True)
                if norm_first:
                    e, inv = e * inv, None
                if n > nv:
                    e = jnp.concatenate([e, jnp.zeros((n - nv, n), F32)], axis=0)
                st[g] = (e.astype(BF16), inv)

            def pv(g):
                nv = len(groups[g]) * L
                n = -(-nv // 16) * 16
                if attn:
                    p, inv = st.pop(g)
                    rb = n if split == 1 else 128 // split
                    vv = _halves(v_v[g, :n // 2, :])
                    o = jnp.concatenate([_dot(p[r:r + rb], vv) for r in range(0, n, rb)], axis=0)[:nv]
                else:
                    inv = None
                    o = (_halves(v_v[g, :n // 2, :]).astype(F32) + _halves(k_v[g, :n // 2, :]).astype(F32) + _halves(q_v[g, :n // 2, :]).astype(F32))[:nv] * 0.01
                if inv is not None:
                    o = o * inv
                for j, h in enumerate(groups[g]):
                    oh = o[j * L:(j + 1) * L]
                    if first:
                        co_v[h] = oh[24:32]
                        o_v[h, :16, :] = _words(jnp.concatenate([oh[:24], oh[32:40]], axis=0).astype(BF16))
                    else:
                        o_v[h, :24, :] = _words(jnp.concatenate([co_v[h], oh], axis=0).astype(BF16))

            mo = 32 if first else 48
            acc = [None] * KD

            def wo(n, h0, h1):
                lhs_o = _halves(jnp.concatenate([o_v[h, :mo // 2, :] for h in range(h0, h1)], axis=1))
                y = _dot(lhs_o, _halves(w_v[rows(WO0 + n * (H * Dh // 2) + h0 * 64, (h1 - h0) * 64), :]))
                if h0 == 0:
                    acc_v[:mo, n * 128:(n + 1) * 128] = y
                elif h1 < H:
                    acc_v[:mo, n * 128:(n + 1) * 128] += y
                else:
                    acc[n] = acc_v[:mo, n * 128:(n + 1) * 128] + y

            tasks = [({"p": proj, "s": scores, "v": pv, "o": wo}[tk[0]],) + tk[1:] for tk in plan(mo)]
            n_wo = 0
            for tk in tasks:
                tk[0](*tk[1:])
                if tk[0] is wo:
                    n_wo += 1
                    if not first and dn_at is not None and 0 <= n_wo - dn_at < KD:
                        filler(n_wo - dn_at)
            if first:
                filler()
            elif dn_at is None:
                for n in range(KD):
                    filler(n)
            return jnp.concatenate(acc, axis=1)

        def base(r0, n):
            return x_v[pl.ds(r0, n), :].astype(F32) + normed(r0, n).astype(F32)

        def macro(t, mem):
            r0 = pl.multiple_of(t * 64, 64)
            slot = t % 2

            @pl.when(t < NF)
            def _():
                for cp in ffn_copies(t, slot):
                    cp.wait()
            hid = []

            def ffn_up():
                if ffn:
                    g = _rnd(_dot(xsel, wg_v[slot])[:16])
                    u = _rnd(_dot(xsel, wu_v[slot])[:16])
                    hid.append(jnp.where(t < NF, _rnd(g * _rnd(jax.nn.sigmoid(g))) * u, 0.0).astype(BF16))

            def ffn_down(n):
                lhs = jnp.concatenate([hid[0]] * (dn_rows // 16), axis=0)
                y_v[:, n * 128:(n + 1) * 128] += _dot(lhs, wd_v[slot, :, n * 128:(n + 1) * 128])[:16]

            ya = step(True, t, mem, ffn_up)
            out_v[pl.ds(r0, 16), :] = (base(r0, 16) + ya[:16]).astype(BF16)
            yb = step(False, t, ya[24:32], ffn_down)
            rest = jnp.concatenate([ya[16:24], yb[:40]], axis=0)
            out_v[pl.ds(r0 + 16, 48), :] = (base(r0 + 16, 48) + rest).astype(BF16)
            out_copy(t).start()

            @pl.when(t + 2 < min(NF, NT_))
            def _():
                for cp in ffn_copies(t + 2, slot):
                    cp.start()
            return yb[40:48]

        jax.lax.fori_loop(0, NT_, macro, mem0_v[0].astype(F32))

        done = pl.ds(0, (NT_ - 1) * 64)
        pltpu.make_async_copy(out_v.at[done, :], out_hbm.at[done, :], sem_out.at[0]).wait()
        late = jnp.maximum(blk0[0], blk0[1]) >= (NT_ - 1) * 64

        @pl.when(late)
        def _():
            out_copy(NT_ - 1).wait()

        y = _rnd(_rnd(y_v[...]) * gate)
        for c in range(2):
            blk = out_v[pl.ds(blk0[c], 16), :].astype(F32)
            out_v[pl.ds(blk0[c], 16), :] = jnp.where(sub == idx[c] - blk0[c], blk + y[c:c + 1], blk).astype(BF16)
        fix = [pltpu.make_async_copy(out_v.at[pl.ds(blk0[c], 16), :], out_hbm.at[pl.ds(blk0[c], 16), :], sem_fix.at[c])
               for c in range(2)]
        fix[0].start()

        @pl.when(blk0[0] != blk0[1])
        def _():
            fix[1].start()
            fix[1].wait()

        @pl.when(jnp.logical_not(late))
        def _():
            out_copy(NT_ - 1).wait()
        fix[0].wait()

    scratch = [
        pltpu.VMEM((1, M, D), BF16),
        pltpu.VMEM((D,), BF16),
        pltpu.VMEM((S + 16, D), BF16),
        pltpu.VMEM((NSEG, 8, D), BF16),
        pltpu.VMEM((KD, NPRE // 2, 128), U32),
        pltpu.VMEM((3, D, HC, 128), BF16),
        pltpu.VMEM((RS0 + 16, 128), U32),
        pltpu.VMEM((NWO, OR, D), BF16),
        pltpu.VMEM((3, H, NPRE // 2, 128), U32),
        pltpu.VMEM((2, D, 128), BF16),
        pltpu.VMEM((2, D, 128), BF16),
        pltpu.VMEM((2, 128, D), BF16),
        pltpu.VMEM((16, D), F32),
        pltpu.VMEM((128, 128), F32),
        pltpu.VMEM((NG, 64, 128), U32),
        pltpu.VMEM((NG, 64, 128), U32),
        pltpu.VMEM((NG, 64, 128), U32),
        pltpu.VMEM((H, 24, 128), U32),
        pltpu.VMEM((H, 8, 128), F32),
        pltpu.VMEM((48, D), F32),
        pltpu.VMEM((S, D), BF16),
        pltpu.SMEM((NHG,), I32),
        pltpu.SemaphoreType.DMA((2,)),
        pltpu.SemaphoreType.DMA((4,)),
        pltpu.SemaphoreType.DMA((4,)),
        pltpu.SemaphoreType.DMA((2,)),
        pltpu.SemaphoreType.DMA((3,)),
        pltpu.SemaphoreType.DMA((NWO,)),
        pltpu.SemaphoreType.DMA((6,)),
        pltpu.SemaphoreType.DMA((2,)),
        pltpu.SemaphoreType.DMA((2,)),
    ]
    return kernel, scratch


def run(A_x, A_mem0, A_Wq, A_Wk, A_Wv, A_Wo, A_seg_len, B_x, B_w_r, B_w_gate, B_w_up, B_w_down, flags=None, nobounds=False, **kw):
    B, S, D = A_x.shape
    _, H, Dh = A_Wq.shape
    M = A_mem0.shape[1]
    F = B_w_gate.shape[1]
    seg = int(A_seg_len)
    kernel, scratch = make_kernel(S, D, H, Dh, M, seg, F, **kw)
    hbm = pl.BlockSpec(memory_space=pl.ANY)
    out = pl.pallas_call(
        kernel,
        out_shape=jax.ShapeDtypeStruct((S, D), A_x.dtype),
        in_specs=[hbm] * 11,
        out_specs=hbm,
        scratch_shapes=scratch,
        compiler_params=pltpu.CompilerParams(vmem_limit_bytes=110 * 1024 * 1024, flags=flags, disable_bounds_checks=nobounds),
    )(A_x.reshape(S, D), A_x.reshape(S // seg, seg, D), A_mem0, A_Wq, A_Wk, A_Wv,
      A_Wo.reshape(H * Dh, D), B_w_r, B_w_gate, B_w_up, B_w_down)
    return out.reshape(B, S, D)


@functools.partial(jax.jit, static_argnames=("A_seg_len",))
def pallas_parallel_sum__memory_aug_recurrent_mem_tr__moe_arch_mod__prompt_kernel(
    A_x, A_mem0, A_Wq, A_Wk, A_Wv, A_Wo, A_seg_len, B_x, B_w_r, B_w_gate, B_w_up, B_w_down,
):
    return run(A_x, A_mem0, A_Wq, A_Wk, A_Wv, A_Wo, A_seg_len, B_x, B_w_r, B_w_gate, B_w_up, B_w_down)
```

```python
import functools
import jax
import jax.numpy as jnp
import numpy as np
import jax.experimental.pallas as pl
import jax.experimental.pallas.tpu as pltpu

F32, BF16, U32, I32 = jnp.float32, jnp.bfloat16, jnp.uint32, jnp.int32
NT = (((1,), (1,)), ((), ()))


def _rnd(v):
    return v.astype(BF16).astype(F32)


def _dot(a, b):
    return jnp.dot(a, b, preferred_element_type=F32)


def _words(v):
    return pltpu.bitcast(v, U32)


def _floats(v):
    return pltpu.bitcast(v, F32)


def _halves(v):
    return pltpu.bitcast(v, BF16)


def make_kernel(S, D, H, Dh, M, SEG, F, nsteps=None, MBQ=64, MBK=128, cuts=(0, 12, 28, 32), early=12, d_ps=220, d_sv=480, d_vo=300, norm_first=True, ffn=True, attn=True, split=1, onebuf=True, pin=True, lag=1, ln_cut=256, dn_at=None, staged=True, up_rows=32, dn_rows=16, nsk=0, ksplit=4, kt=0, U=1, GS=2):
    assert (Dh, M, SEG) == (128, 8, 32) and D % 128 == 0 and F % 128 == 0 and S % 64 == 0
    KD, NF = D // 128, F // 128
    L = M + SEG
    NSEG = S // SEG
    NMAC = S // 64
    HC = 8
    NHG = H // HC
    OR = 512
    NWO = -(-(H * Dh // OR) // (NHG - 1))
    NPRE = NSEG * 8
    scale = Dh ** -0.5
    groups = [list(range(g, min(g + GS, H))) for g in range(0, H, GS)]
    NG = len(groups)
    NT_ = (NMAC if nsteps is None else nsteps) // U
    FB = 128 * U
    NF = F // FB
    PR = 64 * U
    WR = D // 2
    WO0 = (3 * H + HC) * WR
    XN0 = WO0 + KD * H * Dh // 2
    RS0 = XN0 + KD * S // 2
    GR = GS * L // 2
    QKV0 = RS0 + 16
    O0 = QKV0 + 3 * NG * GR
    CO0 = O0 + H * 24
    ACC0 = CO0 + H * 8
    FILL0 = ACC0 + KD * 48
    eps = float(np.asarray(1e-5, dtype=BF16).astype(np.float32))
    neg = float(np.asarray(-1e9, dtype=BF16).astype(np.float32))

    def plan(mo):
        projs = [("p", m, h) for g in groups for m in (1, 0, 2) for h in g]
        outs = [("o", n, h0, h1) for h0, h1 in zip(cuts[:-1], cuts[1:]) for n in range(KD)]
        now, done, order = 0, {}, []
        ns = nv = 0
        while projs or outs or nv < NG:
            due = []
            if nv < ns and ("p", 2, groups[nv][-1]) in done:
                due.append((max(done["s", nv] + d_sv, done["p", 2, groups[nv][-1]] + d_ps), ("v", nv)))
            if ns < NG and ("p", 0, groups[ns][-1]) in done:
                due.append((done["p", 0, groups[ns][-1]] + d_ps, ("s", ns)))
            if outs and ("v", (outs[0][3] - 1) // GS) in done and (not projs or outs[0][3] <= early):
                due.append((done["v", (outs[0][3] - 1) // GS] + d_vo, outs[0]))
            ready = [d for d in due if d[0] <= now]
            task = ready[0][1] if ready else projs[0] if projs else min(due)[1]
            if task[0] == "p":
                projs.pop(0)
                now += KD * 32 // 4
            elif task[0] == "o":
                outs.pop(0)
                now += (task[3] - task[2]) * mo // 4
            else:
                now += GS * L // 4
                ns, nv = ns + (task[0] == "s"), nv + (task[0] == "v")
            done[task] = now
            order.append(task)
        return order

    def kernel(x_hbm, x3_hbm, mem0_hbm, wq_hbm, wk_hbm, wv_hbm, wo_hbm, wr_hbm, wg_hbm, wu_hbm, wd_hbm,
               out_hbm,
               mem0_v, wr_v, x_v, xp_v, xpre_v, st_v, w_v, wost_v, pre_v, wg_v, wu_v, wd_v, y_v,
               out_v, tab_s,
               sem_in, sem_xp, sem_q0, sem_x, sem_st, sem_wo, sem_f, sem_out, sem_fix):
        srcs = (wq_hbm, wk_hbm, wv_hbm)
        WOFF = (2 * H, 0, H)
        XR = S // NHG

        def st_copy(m, hg, zero=0):
            return pltpu.make_async_copy(
                srcs[m].at[:, pl.ds(pl.multiple_of(hg * HC, HC), HC), :], st_v.at[m + zero], sem_st.at[m])

        def x_copy(hg, part):
            a, b = ((0, ln_cut), (ln_cut, XR))[part]
            rows = pl.ds(pl.multiple_of(hg * XR + a, 16), b - a)
            return pltpu.make_async_copy(x_hbm.at[rows, :], x_v.at[rows, :], sem_x.at[part])

        def wo_block(hg, j):
            return jnp.minimum(hg * NWO + j, H * Dh // OR - 1)

        def wo_copy(hg, j):
            rows = pl.ds(pl.multiple_of(wo_block(hg, j) * OR, OR), OR)
            return pltpu.make_async_copy(wo_hbm.at[rows, :], wost_v.at[j], sem_wo.at[j])

        def ffn_copies(j, slot):
            f0 = pl.ds(pl.multiple_of(j * FB, FB), FB)
            return (pltpu.make_async_copy(wg_hbm.at[:, f0], wg_v.at[slot], sem_f.at[3 * slot]),
                    pltpu.make_async_copy(wu_hbm.at[:, f0], wu_v.at[slot], sem_f.at[3 * slot + 1]),
                    pltpu.make_async_copy(wd_hbm.at[f0, :], wd_v.at[slot], sem_f.at[3 * slot + 2]))

        def out_copy(t):
            rows = pl.ds(pl.multiple_of(t * PR, PR), PR)
            last = jnp.where(t == NT_ - 1, 1, 0)
            return pltpu.make_async_copy(out_v.at[rows, :], out_hbm.at[rows, :], sem_out.at[last])

        def layernorm(xf):
            mean = jnp.sum(xf, axis=-1, keepdims=True) * (1.0 / D)
            cen = xf - mean
            var = jnp.sum(cen * cen, axis=-1, keepdims=True) * (1.0 / D)
            den = _rnd(jnp.sqrt(_rnd(_rnd(var) + eps)))
            return (_rnd(xf - _rnd(mean)) * (1.0 / den)).astype(BF16)

        sub8 = jax.lax.broadcasted_iota(I32, (8, 128), 0)

        def rows(start, n):
            return pl.ds(start if isinstance(start, int) else pl.multiple_of(start, 8), n)

        def weight(m, h, k0=0, k1=KD):
            return _halves(w_v[rows((WOFF[m] + h) * WR + k0 * 64, (k1 - k0) * 64), :])

        def normed(t, r, n):
            return _halves(jnp.concatenate(
                [w_v[rows(XN0 + t * (KD * 32) + k * 32 + (r >> 1), n // 2), :] for k in range(KD)], axis=1))

        def relayout(m, h0):
            def piece(d0):
                x = _words(st_v[m, pl.ds(d0, 16)].reshape(16 * HC, 128))
                v = [x[8 * i:8 * i + 8] for i in range(8)]
                for bit in (1, 2, 4):
                    keep = (sub8 & bit) == 0
                    for i in range(8):
                        if not i & bit:
                            p, q = v[i], v[i + bit]
                            v[i] = jnp.where(keep, p, pltpu.roll(q, bit, 0))
                            v[i + bit] = jnp.where(keep, pltpu.roll(p, 8 - bit, 0), q)
                for j in range(HC // 2):
                    even, odd = v[j], v[j + 4]
                    at = (WOFF[m] + h0 + 2 * j) * WR + d0 // 2
                    w_v[rows(at, 8), :] = (even & 0xFFFF) | (odd << 16)
                    w_v[rows(at + WR, 8), :] = (even >> 16) | (odd & np.uint32(0xFFFF0000))
            return [functools.partial(piece, d0) for d0 in range(0, D, 16)]

        def weave(*jobs):
            order = sorted(((i + 0.5) / len(js), n, i) for n, js in enumerate(jobs) for i in range(len(js)))
            for _, n, i in order:
                jobs[n][i]()

        xp_cps = [pltpu.make_async_copy(x3_hbm.at[pl.ds(i * (NSEG // 4), NSEG // 4), pl.ds(0, 8), :],
                                        xp_v.at[pl.ds(i * (NSEG // 4), NSEG // 4)], sem_xp.at[i]) for i in range(4)]
        q0_cps = [pltpu.make_async_copy(wq_hbm.at[pl.ds(i * (D // 4), D // 4), pl.ds(0, HC), :],
                                        st_v.at[0, pl.ds(i * (D // 4), D // 4)], sem_q0.at[i]) for i in range(4)]
        in_cps = [pltpu.make_async_copy(wr_hbm, wr_v, sem_in.at[0]), pltpu.make_async_copy(mem0_hbm, mem0_v, sem_in.at[1])]
        for cp in xp_cps[:2] + in_cps:
            cp.start()

        ri = jax.lax.broadcasted_iota(I32, (128, 128), 0)
        ci = jax.lax.broadcasted_iota(I32, (128, 128), 1)
        hr = (ri >= L).astype(I32) + (ri >= 2 * L).astype(I32) + (ri >= 3 * L).astype(I32)
        hc = (ci >= L).astype(I32) + (ci >= 2 * L).astype(I32) + (ci >= 3 * L).astype(I32)
        tr, tc = ri - hr * L, ci - hc * L
        vis = (tr >= SEG) | (tc >= SEG) | (tc <= tr)
        w_v[rows(FILL0, 128), :] = _words(jnp.where(hr == hc, jnp.where(vis, 0.0, neg), -jnp.inf))
        y_v[...] = jnp.zeros(y_v.shape, F32)
        for i in range(NHG):
            tab_s[i] = i

        def pre_ln(i, c):
            xf = jnp.concatenate([xp_v[i * 8 + j].astype(F32) for j in range(8)], axis=0)
            w = _words(layernorm(xf))
            for k in range(KD):
                xpre_v[k, pl.ds(pl.multiple_of(i * 32, 32), 32), :] = w[:, k * 128:(k + 1) * 128]
            return c
        ahead = [xp_cps[2:] + q0_cps[:1], [], q0_cps[1:2], q0_cps[2:3], q0_cps[3:], [], [st_copy(1, 0), x_copy(0, 0)], []]
        for i, cp in enumerate(xp_cps):
            cp.wait()
            for nxt in ahead[i]:
                nxt.start()
            jax.lax.fori_loop(i * (NSEG // 32), (i + 1) * (NSEG // 32), pre_ln, 0)
        first_q = relayout(0, 0)
        for i, cp in enumerate(q0_cps):
            cp.wait()
            for nxt in ahead[4 + i]:
                nxt.start()
            weave(first_q[i * (len(first_q) // 4):(i + 1) * (len(first_q) // 4)])


        lane = jax.lax.broadcasted_iota(I32, (16, 128), 1)
        sub = jax.lax.broadcasted_iota(I32, (16, 1), 0)

        def project_pre(m, h0, zero=None):
            MB = MBQ if zero is None else MBK

            def piece(hh, r):
                lhs = _halves(jnp.concatenate([xpre_v[k, r // 2:(r + MB) // 2, :] for k in range(KD)], axis=1))
                y = _dot(lhs, weight(m, h0 + hh)).astype(BF16)
                pre_v[r // 16:(r + MB) // 16, m, h0 + hh] = _words(y).reshape(MB // 16, 8, 128)
                if zero is not None:
                    x_v[pl.ds(pl.multiple_of(S + zero, 16), 16), :128] = y[:16]
            return [functools.partial(piece, hh, r) for hh in range(HC) for r in range(0, NPRE, MB)]

        def norm_rows(hg, sg, a, b, score):
            r0 = hg * XR
            held = {}

            def load(r):
                return x_v[pl.ds(pl.multiple_of(r0 + r, 16), 16), :].astype(F32)

            def mean(r):
                held[r] = jnp.sum(load(r), axis=-1, keepdims=True) * (1.0 / D)

            def spread(r):
                cen = load(r) - held[r]
                var = jnp.sum(cen * cen, axis=-1, keepdims=True) * (1.0 / D)
                held[r] = _rnd(held[r]), 1.0 / _rnd(jnp.sqrt(_rnd(_rnd(var) + eps)))

            def apply(r):
                mu, inv = held[r]
                xn = (_rnd(load(r) - mu) * inv).astype(BF16)
                held[r] = _words(xn), _rnd(jnp.sum(xn.astype(F32) * wr, axis=-1, keepdims=True))

            def whole(r):
                xn = layernorm(load(r))
                held[r] = _words(xn), _rnd(jnp.sum(xn.astype(F32) * wr, axis=-1, keepdims=True))

            def commit(r):
                xw = held[r][0]
                for k in range(KD):
                    w_v[rows(XN0 + (sg * (XR // 64) + r // 64) * (KD * 32) + k * 32 + r % 64 // 2, 8), :] = xw[:, k * 128:(k + 1) * 128]

            def note(r):
                score[0] = jnp.where(lane == (r0 + r) // 16, held.pop(r)[1], score[0])
                w_v[rows(RS0 + (sg - hg) * 8, 16), :] = pltpu.bitcast(score[0], U32)

            rs = list(range(a, b, 16))
            stages = [(mean, 0), (spread, 1), (apply, 2), (commit, 2 + lag), (note, 3)] if staged else [(whole, 0), (commit, lag), (note, lag)]
            depth = max(d for _, d in stages)
            nop = [lambda: None]
            return [nop * d + [functools.partial(f, r) for r in rs] + nop * (depth - d) for f, d in stages]

        def repack_wo(hg):
            def piece(j, r):
                w = _words(wost_v[j, r:r + 32, :])
                for n in range(KD):
                    w_v[rows(WO0 + n * (H * Dh // 2) + wo_block(hg, j) * (OR // 2) + r // 2, 16), :] = w[:, n * 128:(n + 1) * 128]
            return [functools.partial(piece, j, r) for j in range(NWO) for r in range(0, OR, 32)]

        dots = project_pre(0, 0)
        weave(dots[:len(dots) // 2])
        st_copy(1, 0).wait()

        @pl.when(tab_s[0] == 0)
        def _():
            st_copy(2, 0).start()
        weave(dots[len(dots) // 2:], relayout(1, tab_s[0]))
        for cp in in_cps:
            cp.wait()
        wr = wr_v[...].astype(F32).reshape(1, D)

        def pre_body(hg, score):
            h0 = pl.multiple_of(hg * HC, HC)
            more = hg + 1 < NHG
            sg = tab_s[hg]
            zero = tab_s[0]
            score = [score]

            def norm(a, b):
                return norm_rows(hg, sg, a, b, score)

            @pl.when(more)
            def _():
                st_copy(0, hg + 1).start()
                wo_copy(hg, 0).start()

            @pl.when(jnp.logical_not(more))
            def _():
                for cp in ffn_copies(0, 0) + ffn_copies(1, 1):
                    cp.start()
            x_copy(hg, 1).start()
            st_copy(2, hg).wait()
            x_copy(hg, 0).wait()
            weave(project_pre(1, h0, zero), relayout(2, sg * HC), *norm(0, ln_cut))

            @pl.when(more)
            def _():
                st_copy(1, hg + 1).start()
                for j in range(1, NWO):
                    wo_copy(hg, j).start()
                st_copy(0, hg + 1).wait()
            x_copy(hg, 1).wait()
            weave(project_pre(2, h0, zero), relayout(0, sg * HC + HC), *norm(ln_cut, XR))

            @pl.when(more)
            def _():
                st_copy(2, hg + 1).start()
                x_copy(hg + 1, 0).start()
                st_copy(1, hg + 1).wait()
                for j in range(NWO):
                    wo_copy(hg, j).wait()
                weave(project_pre(0, h0 + HC), relayout(1, sg * HC + HC), repack_wo(sg))
            return score[0]

        score = jax.lax.fori_loop(0, NHG, pre_body, jnp.zeros((16, 128), F32))

        def first_max(key, free):
            top = jnp.max(jnp.max(key, axis=1, keepdims=True), axis=0, keepdims=True)
            first = jnp.where((key == top) & free, tok_id, float(S))
            return top, jnp.min(jnp.min(first, axis=1, keepdims=True), axis=0, keepdims=True)

        tok_id = (lane * 16 + sub).astype(F32)
        key = jnp.where(score == score, score, -jnp.inf)
        m1, i1 = first_max(key, tok_id >= 0)
        m2, i2 = first_max(jnp.where(tok_id == i1, -jnp.inf, key), tok_id != i1)
        idx = [i.astype(I32)[0, 0] for i in (i1, i2)]
        gate = jnp.where(sub == 0, _rnd(jax.nn.sigmoid(m1)), _rnd(jax.nn.sigmoid(m2)))
        xsel = jnp.zeros((16, D), F32)
        blk0 = []
        for c in range(2):
            b = pl.multiple_of(idx[c] & ~15, 16)
            blk0.append(b)
            rowv = jnp.sum(jnp.where(sub == idx[c] - b, normed(b >> 6, b & 63, 16).astype(F32), 0.0), axis=0, keepdims=True)
            xsel = jnp.where(sub == c, rowv, xsel)
        xsel = jnp.concatenate([xsel] * (up_rows // 16), axis=0).astype(BF16)

        def step(first, t, mem, filler):
            xs = normed(t, 0 if first else 32, 32)
            lhs = jnp.concatenate(
                [jnp.concatenate([mem, xs[:16].astype(F32)[8:]], axis=0).astype(BF16), xs[16:]], axis=0)
            pend = {}

            part = {}

            def proj_head(m, h):
                part[m, h] = _dot(lhs[:, :ksplit * 128], weight(m, h, 0, ksplit))

            def proj(m, h):
                if (m, h) in part:
                    y = part.pop((m, h)) + _dot(lhs[:, ksplit * 128:], weight(m, h, ksplit, KD))
                else:
                    y = _dot(lhs, weight(m, h))
                pre = _halves(pre_v[t, m, h]).astype(F32)
                tok = jnp.concatenate([pre[:8] if first else pre[8:], y[8:], y[:8]], axis=0)
                g, j = divmod(h, GS)
                pend.setdefault((m, g), []).append(tok)
                if j == len(groups[g]) - 1:
                    toks = pend.pop((m, g))
                    w_v[rows(QKV0 + (m * NG + g) * GR, GR), :] = _words(jnp.concatenate(toks, axis=0).astype(BF16))

            def tokens(m, g):
                return _halves(w_v[rows(QKV0 + (m * NG + g) * GR, GR), :])

            st = {}

            def scores(g):
                n = GS * L
                s = jax.lax.dot_general(tokens(0, g), tokens(1, g), NT, preferred_element_type=F32)
                fill = _floats(w_v[rows(FILL0, n), :])[:, :n]
                s = jnp.where(fill == 0.0, s * scale, fill)
                e = jnp.exp(s - jnp.max(s, axis=-1, keepdims=True))
                st[g] = (e * (1.0 / jnp.sum(e, axis=-1, keepdims=True))).astype(BF16)

            def pv(g):
                o = _dot(st.pop(g), tokens(2, g))
                for j, h in enumerate(groups[g]):
                    oh = o[j * L:(j + 1) * L]
                    if first:
                        w_v[rows(CO0 + h * 8, 8), :] = _words(oh[24:32])
                        w_v[rows(O0 + h * 24, 16), :] = _words(jnp.concatenate([oh[:24], oh[32:40]], axis=0).astype(BF16))
                    else:
                        held = _floats(w_v[rows(CO0 + h * 8, 8), :])
                        w_v[rows(O0 + h * 24, 24), :] = _words(jnp.concatenate([held, oh], axis=0).astype(BF16))

            mo = 32 if first else 48
            acc = [None] * KD

            def wo(n, h0, h1):
                lhs_o = _halves(jnp.concatenate([w_v[rows(O0 + h * 24, mo // 2), :] for h in range(h0, h1)], axis=1))
                y = _dot(lhs_o, _halves(w_v[rows(WO0 + n * (H * Dh // 2) + h0 * 64, (h1 - h0) * 64), :]))
                if h0 > 0:
                    y = _floats(w_v[rows(ACC0 + n * 48, mo), :]) + y
                if h1 < H:
                    w_v[rows(ACC0 + n * 48, mo), :] = _words(y)
                else:
                    acc[n] = y

            tasks = [({"p": proj, "s": scores, "v": pv, "o": wo}[tk[0]],) + tk[1:] for tk in plan(mo)]
            if not first:
                for tk in tasks[:nsk]:
                    proj_head(*tk[1:])
            for tk in tasks:
                tk[0](*tk[1:])
            filler()
            return jnp.concatenate(acc, axis=1)

        def base(t, r, n):
            return x_v[pl.ds(pl.multiple_of(t * 64 + r, 16), n), :].astype(F32) + normed(t, r, n).astype(F32)

        def macro(t, mem):
            slot = t % 2

            @pl.when(t < NF)
            def _():
                for cp in ffn_copies(t, slot):
                    cp.wait()
            hid = []

            def ffn_up(c):
                g = _rnd(_dot(xsel, wg_v[slot, :, c * 128:(c + 1) * 128])[:16])
                u = _rnd(_dot(xsel, wu_v[slot, :, c * 128:(c + 1) * 128])[:16])
                hid.append(jnp.where(t < NF, _rnd(g * _rnd(jax.nn.sigmoid(g))) * u, 0.0).astype(BF16))

            def ffn_down():
                lhs = jnp.concatenate([jnp.concatenate(hid, axis=1)] * (dn_rows // 16), axis=0)
                y_v[...] += _dot(lhs, wd_v[slot])[:16]

            fillers = [functools.partial(ffn_up, c) for c in range(U)] + [ffn_down] + [lambda: None] * U
            for u in range(U):
                r0 = pl.multiple_of((t * U + u) * 64, 64)
                ya = step(True, t * U + u, mem, fillers[2 * u])
                out_v[pl.ds(r0, 16), :] = (base(t * U + u, 0, 16) + ya[:16]).astype(BF16)
                yb = step(False, t * U + u, ya[24:32], fillers[2 * u + 1])
                rest = jnp.concatenate([ya[16:24], yb[:40]], axis=0)
                out_v[pl.ds(r0 + 16, 48), :] = (base(t * U + u, 16, 48) + rest).astype(BF16)
                mem = yb[40:48]
            out_copy(t).start()

            @pl.when(t + 2 < min(NF, NT_))
            def _():
                for cp in ffn_copies(t + 2, slot):
                    cp.start()
            return mem

        jax.lax.fori_loop(0, NT_, macro, mem0_v[0].astype(F32))

        done = pl.ds(0, (NT_ - 1) * PR)
        pltpu.make_async_copy(out_v.at[done, :], out_hbm.at[done, :], sem_out.at[0]).wait()
        late = jnp.maximum(blk0[0], blk0[1]) >= (NT_ - 1) * PR

        @pl.when(late)
        def _():
            out_copy(NT_ - 1).wait()

        y = _rnd(_rnd(y_v[...]) * gate)
        for c in range(2):
            blk = out_v[pl.ds(blk0[c], 16), :].astype(F32)
            out_v[pl.ds(blk0[c], 16), :] = jnp.where(sub == idx[c] - blk0[c], blk + y[c:c + 1], blk).astype(BF16)
        fix = [pltpu.make_async_copy(out_v.at[pl.ds(blk0[c], 16), :], out_hbm.at[pl.ds(blk0[c], 16), :], sem_fix.at[c])
               for c in range(2)]
        fix[0].start()

        @pl.when(blk0[0] != blk0[1])
        def _():
            fix[1].start()
            fix[1].wait()

        @pl.when(jnp.logical_not(late))
        def _():
            out_copy(NT_ - 1).wait()
        fix[0].wait()

    scratch = [
        pltpu.VMEM((1, M, D), BF16),
        pltpu.VMEM((D,), BF16),
        pltpu.VMEM((S + 16, D), BF16),
        pltpu.VMEM((NSEG, 8, D), BF16),
        pltpu.VMEM((KD, NPRE // 2, 128), U32),
        pltpu.VMEM((3, D, HC, 128), BF16),
        pltpu.VMEM((FILL0 + 128, 128), U32),
        pltpu.VMEM((NWO, OR, D), BF16),
        pltpu.VMEM((NMAC, 3, H, 8, 128), U32),
        pltpu.VMEM((2, D, FB), BF16),
        pltpu.VMEM((2, D, FB), BF16),
        pltpu.VMEM((2, FB, D), BF16),
        pltpu.VMEM((16, D), F32),
        pltpu.VMEM((S, D), BF16),
        pltpu.SMEM((NHG,), I32),
        pltpu.SemaphoreType.DMA((2,)),
        pltpu.SemaphoreType.DMA((4,)),
        pltpu.SemaphoreType.DMA((4,)),
        pltpu.SemaphoreType.DMA((2,)),
        pltpu.SemaphoreType.DMA((3,)),
        pltpu.SemaphoreType.DMA((NWO,)),
        pltpu.SemaphoreType.DMA((6,)),
        pltpu.SemaphoreType.DMA((2,)),
        pltpu.SemaphoreType.DMA((2,)),
    ]
    return kernel, scratch


def run(A_x, A_mem0, A_Wq, A_Wk, A_Wv, A_Wo, A_seg_len, B_x, B_w_r, B_w_gate, B_w_up, B_w_down, flags=None, nobounds=True, **kw):
    B, S, D = A_x.shape
    _, H, Dh = A_Wq.shape
    M = A_mem0.shape[1]
    F = B_w_gate.shape[1]
    seg = int(A_seg_len)
    kernel, scratch = make_kernel(S, D, H, Dh, M, seg, F, **kw)
    hbm = pl.BlockSpec(memory_space=pl.ANY)
    out = pl.pallas_call(
        kernel,
        out_shape=jax.ShapeDtypeStruct((S, D), A_x.dtype),
        in_specs=[hbm] * 11,
        out_specs=hbm,
        scratch_shapes=scratch,
        compiler_params=pltpu.CompilerParams(vmem_limit_bytes=110 * 1024 * 1024, flags=flags, disable_bounds_checks=nobounds),
    )(A_x.reshape(S, D), A_x.reshape(S // seg, seg, D), A_mem0, A_Wq, A_Wk, A_Wv,
      A_Wo.reshape(H * Dh, D), B_w_r, B_w_gate, B_w_up, B_w_down)
    return out.reshape(B, S, D)


@functools.partial(jax.jit, static_argnames=("A_seg_len",))
def pallas_parallel_sum__memory_aug_recurrent_mem_tr__moe_arch_mod__prompt_kernel(
    A_x, A_mem0, A_Wq, A_Wk, A_Wv, A_Wo, A_seg_len, B_x, B_w_r, B_w_gate, B_w_up, B_w_down,
):
    return run(A_x, A_mem0, A_Wq, A_Wk, A_Wv, A_Wo, A_seg_len, B_x, B_w_r, B_w_gate, B_w_up, B_w_down)
```

```python
import functools

import jax
import jax.numpy as jnp
import numpy as np
import jax.experimental.pallas as pl
import jax.experimental.pallas.tpu as pltpu

F32, BF16, U32, I32 = jnp.float32, jnp.bfloat16, jnp.uint32, jnp.int32
CONTRACT_LAST = (((1,), (1,)), ((), ()))


def _rnd(v):
    return v.astype(BF16).astype(F32)


def _dot(a, b):
    return jnp.dot(a, b, preferred_element_type=F32)


def _words(v):
    return pltpu.bitcast(v, U32)


def _floats(v):
    return pltpu.bitcast(v, F32)


def _halves(v):
    return pltpu.bitcast(v, BF16)


def _rows(start, n):
    return pl.ds(start if isinstance(start, int) else pl.multiple_of(start, 8), n)


def _weave(*jobs):
    order = sorted(((i + 0.5) / len(js), n, i) for n, js in enumerate(jobs) for i in range(len(js)))
    for _, n, i in order:
        jobs[n][i]()


def _plan(heads, pair, kd, out_rows, pair_rows, cuts, early, d_proj, d_soft, d_mix):
    pairs = [range(g, g + pair) for g in range(0, heads, pair)]
    projs = [("project", m, h) for g in pairs for m in (1, 0, 2) for h in g]
    outs = [("output", n, h0, h1) for h0, h1 in zip(cuts[:-1], cuts[1:]) for n in range(kd)]
    now, done, order = 0, {}, []
    ns = nv = 0
    while projs or outs or nv < len(pairs):
        due = []
        if nv < ns and ("project", 2, pairs[nv][-1]) in done:
            due.append((max(done["score", nv] + d_soft, done["project", 2, pairs[nv][-1]] + d_proj), ("mix", nv)))
        if ns < len(pairs) and ("project", 0, pairs[ns][-1]) in done:
            due.append((done["project", 0, pairs[ns][-1]] + d_proj, ("score", ns)))
        if outs and ("mix", (outs[0][3] - 1) // pair) in done and (not projs or outs[0][3] <= early):
            due.append((done["mix", (outs[0][3] - 1) // pair] + d_mix, outs[0]))
        ready = [d for d in due if d[0] <= now]
        task = ready[0][1] if ready else projs[0] if projs else min(due)[1]
        if task[0] == "project":
            projs.pop(0)
            now += kd * 32 // 4
        elif task[0] == "output":
            outs.pop(0)
            now += (task[3] - task[2]) * out_rows // 4
        else:
            now += pair_rows // 4
            ns, nv = ns + (task[0] == "score"), nv + (task[0] == "mix")
        done[task] = now
        order.append(task)
    return order


def make_kernel(S, D, H, Dh, M, SEG, F, cuts=(0, 12, 28, 32), early=12, d_proj=220, d_soft=480, d_mix=240,
                MBQ=64, MBK=128, ln_cut=256, first_cut=32):
    assert (Dh, M, SEG) == (128, 8, 32) and D % 128 == 0 and F % 128 == 0 and S == 64 * H and F // 128 <= S // 64
    KD, NF = D // 128, F // 128
    L = M + SEG
    NSEG = S // SEG
    NPASS = S // 64
    NPRE = NSEG * 8
    HC = 8
    NHG = H // HC
    XR = S // NHG
    OR = 512
    NWO = -(-(H * Dh // OR) // (NHG - 1))
    PAIR = 2
    scale = Dh ** -0.5
    eps = float(np.asarray(1e-5, dtype=BF16).astype(np.float32))
    hidden = float(np.asarray(-1e9, dtype=BF16).astype(np.float32))

    WR = D // 2
    WOFF = (2 * H, 0, H)
    WO0 = (3 * H + HC) * WR
    XN0 = WO0 + KD * H * Dh // 2
    RS0 = XN0 + KD * S // 2
    GR = PAIR * L // 2
    QKV0 = RS0 + 16
    O0 = QKV0 + 3 * H // PAIR * GR
    CO0 = O0 + H * 24
    ACC0 = CO0 + H * 8
    FILL0 = ACC0 + KD * 48

    def kernel(x_hbm, x3_hbm, mem0_hbm, wq_hbm, wk_hbm, wv_hbm, wo_hbm, wr_hbm, wg_hbm, wu_hbm, wd_hbm,
               out_hbm,
               mem0_v, wr_v, x_v, xp_v, xpre_v, st_v, w_v, wost_v, pre_v, wg_v, wu_v, wd_v, y_v, out_v, tab_s,
               sem_in, sem_xp, sem_q0, sem_x, sem_st, sem_wo, sem_f, sem_out, sem_fix):
        sub8 = jax.lax.broadcasted_iota(I32, (8, 128), 0)
        sub = jax.lax.broadcasted_iota(I32, (16, 1), 0)
        lane = jax.lax.broadcasted_iota(I32, (16, 128), 1)

        def st_copy(m, hg):
            heads = pl.ds(pl.multiple_of(hg * HC, HC), HC)
            return pltpu.make_async_copy((wq_hbm, wk_hbm, wv_hbm)[m].at[:, heads, :], st_v.at[m], sem_st.at[m])

        def x_copy(hg, part):
            a, b = ((0, ln_cut), (ln_cut, XR))[part]
            rows = pl.ds(pl.multiple_of(hg * XR + a, 16), b - a)
            return pltpu.make_async_copy(x_hbm.at[rows, :], x_v.at[rows, :], sem_x.at[part])

        def wo_block(hg, j):
            return jnp.minimum(hg * NWO + j, H * Dh // OR - 1)

        def wo_copy(hg, j):
            rows = pl.ds(pl.multiple_of(wo_block(hg, j) * OR, OR), OR)
            return pltpu.make_async_copy(wo_hbm.at[rows, :], wost_v.at[j], sem_wo.at[j])

        def ffn_copies(j, slot):
            cols = pl.ds(pl.multiple_of(j * 128, 128), 128)
            return (pltpu.make_async_copy(wg_hbm.at[:, cols], wg_v.at[slot], sem_f.at[3 * slot]),
                    pltpu.make_async_copy(wu_hbm.at[:, cols], wu_v.at[slot], sem_f.at[3 * slot + 1]),
                    pltpu.make_async_copy(wd_hbm.at[cols, :], wd_v.at[slot], sem_f.at[3 * slot + 2]))

        def out_copy(t):
            rows = pl.ds(pl.multiple_of(t * 64, 64), 64)
            return pltpu.make_async_copy(out_v.at[rows, :], out_hbm.at[rows, :],
                                         sem_out.at[jnp.where(t == NPASS - 1, 1, 0)])

        def row_mean(v):
            return jnp.sum(v, axis=-1, keepdims=True) * (1.0 / D)

        def inv_spread(v, mean):
            cen = v - mean
            return 1.0 / _rnd(jnp.sqrt(_rnd(_rnd(row_mean(cen * cen)) + eps)))

        def normalise(v, mean, inv):
            return (_rnd(v - _rnd(mean)) * inv).astype(BF16)

        def weight(m, h):
            return _halves(w_v[_rows((WOFF[m] + h) * WR, WR), :])

        def normed(t, r, n):
            return _halves(jnp.concatenate(
                [w_v[_rows(XN0 + t * (KD * 32) + k * 32 + (r >> 1), n // 2), :] for k in range(KD)], axis=1))

        def relayout(m, h0):
            def piece(d0):
                x = _words(st_v[m, pl.ds(d0, 16)].reshape(16 * HC, 128))
                v = [x[8 * i:8 * i + 8] for i in range(8)]
                for bit in (1, 2, 4):
                    keep = (sub8 & bit) == 0
                    for i in range(8):
                        if not i & bit:
                            p, q = v[i], v[i + bit]
                            v[i] = jnp.where(keep, p, pltpu.roll(q, bit, 0))
                            v[i + bit] = jnp.where(keep, pltpu.roll(p, 8 - bit, 0), q)
                for j in range(HC // 2):
                    even, odd = v[j], v[j + 4]
                    at = (WOFF[m] + h0 + 2 * j) * WR + d0 // 2
                    w_v[_rows(at, 8), :] = (even & 0xFFFF) | (odd << 16)
                    w_v[_rows(at + WR, 8), :] = (even >> 16) | (odd & np.uint32(0xFFFF0000))
            return [functools.partial(piece, d0) for d0 in range(0, D, 16)]

        def repack_wo(hg):
            def piece(j, r):
                w = _words(wost_v[j, r:r + 32, :])
                for n in range(KD):
                    at = WO0 + n * (H * Dh // 2) + wo_block(hg, j) * (OR // 2) + r // 2
                    w_v[_rows(at, 16), :] = w[:, n * 128:(n + 1) * 128]
            return [functools.partial(piece, j, r) for j in range(NWO) for r in range(0, OR, 32)]

        def project_pre(m, h0, zero=None):
            mb = MBQ if zero is None else MBK

            def piece(hh, r):
                lhs = _halves(jnp.concatenate([xpre_v[k, r // 2:(r + mb) // 2, :] for k in range(KD)], axis=1))
                y = _dot(lhs, weight(m, h0 + hh)).astype(BF16)
                pre_v[r // 16:(r + mb) // 16, m, h0 + hh] = _words(y).reshape(mb // 16, 8, 128)
                if zero is not None:
                    x_v[pl.ds(pl.multiple_of(S + zero, 16), 16), :128] = y[:16]
            return [functools.partial(piece, hh, r) for hh in range(HC) for r in range(0, NPRE, mb)]

        def norm_and_score(hg, sg, a, b, score):
            held = {}

            def load(r):
                return x_v[pl.ds(pl.multiple_of(hg * XR + r, 16), 16), :].astype(F32)

            def first(r):
                held[r] = row_mean(load(r))

            def second(r):
                held[r] = held[r], inv_spread(load(r), held[r])

            def third(r):
                xn = normalise(load(r), *held[r])
                held[r] = _words(xn), _rnd(jnp.sum(xn.astype(F32) * wr, axis=-1, keepdims=True))

            def commit(r):
                xw, sc = held.pop(r)
                for k in range(KD):
                    at = XN0 + (sg * (XR // 64) + r // 64) * (KD * 32) + k * 32 + r % 64 // 2
                    w_v[_rows(at, 8), :] = xw[:, k * 128:(k + 1) * 128]
                score[0] = jnp.where(lane == (hg * XR + r) // 16, sc, score[0])
                w_v[_rows(RS0 + (sg - hg) * 8, 16), :] = _words(score[0])

            stages = (first, second, third, commit)
            nop = [lambda: None]
            return [nop * d + [functools.partial(f, r) for r in range(a, b, 16)] + nop * (len(stages) - 1 - d)
                    for d, f in enumerate(stages)]

        xp_cps = [pltpu.make_async_copy(x3_hbm.at[pl.ds(i * (NSEG // 4), NSEG // 4), pl.ds(0, 8), :],
                                        xp_v.at[pl.ds(i * (NSEG // 4), NSEG // 4)], sem_xp.at[i]) for i in range(4)]
        q0_cps = [pltpu.make_async_copy(wq_hbm.at[pl.ds(i * (D // 4), D // 4), pl.ds(0, HC), :],
                                        st_v.at[0, pl.ds(i * (D // 4), D // 4)], sem_q0.at[i]) for i in range(4)]
        in_cps = [pltpu.make_async_copy(wr_hbm, wr_v, sem_in.at[0]),
                  pltpu.make_async_copy(mem0_hbm, mem0_v, sem_in.at[1])]
        ahead = [xp_cps[2:] + q0_cps[:1], [], q0_cps[1:2], q0_cps[2:3],
                 q0_cps[3:], [], [st_copy(1, 0), x_copy(0, 0)], []]
        for cp in xp_cps[:2] + in_cps:
            cp.start()

        ri = jax.lax.broadcasted_iota(I32, (PAIR * L, 128), 0)
        ci = jax.lax.broadcasted_iota(I32, (PAIR * L, 128), 1)
        tr, tc = jnp.where(ri >= L, ri - L, ri), jnp.where(ci >= L, ci - L, ci)
        visible = (tr >= SEG) | (tc >= SEG) | (tc <= tr)
        w_v[_rows(FILL0, PAIR * L), :] = _words(
            jnp.where(ri - tr == ci - tc, jnp.where(visible, 0.0, hidden), -jnp.inf))
        y_v[...] = jnp.zeros(y_v.shape, F32)
        for i in range(NHG):
            tab_s[i] = i

        def pre_norm(i, carry):
            v = jnp.concatenate([xp_v[i * 8 + j].astype(F32) for j in range(8)], axis=0)
            mean = row_mean(v)
            w = _words(normalise(v, mean, inv_spread(v, mean)))
            for k in range(KD):
                xpre_v[k, pl.ds(pl.multiple_of(i * 32, 32), 32), :] = w[:, k * 128:(k + 1) * 128]
            return carry

        for i, cp in enumerate(xp_cps):
            cp.wait()
            for nxt in ahead[i]:
                nxt.start()
            jax.lax.fori_loop(i * (NSEG // 32), (i + 1) * (NSEG // 32), pre_norm, 0)
        pieces = relayout(0, 0)
        for i, cp in enumerate(q0_cps):
            cp.wait()
            for nxt in ahead[4 + i]:
                nxt.start()
            _weave(pieces[i * (len(pieces) // 4):(i + 1) * (len(pieces) // 4)])

        dots = project_pre(0, 0)
        _weave(dots[:first_cut])
        st_copy(1, 0).wait()

        @pl.when(tab_s[0] == 0)
        def _():
            st_copy(2, 0).start()
        _weave(dots[first_cut:], relayout(1, tab_s[0]))
        for cp in in_cps:
            cp.wait()
        wr = wr_v[...].astype(F32).reshape(1, D)

        def pre_body(hg, score):
            h0 = pl.multiple_of(hg * HC, HC)
            more = hg + 1 < NHG
            sg = tab_s[hg]
            zero = tab_s[0]
            score = [score]

            @pl.when(more)
            def _():
                st_copy(0, hg + 1).start()
                wo_copy(hg, 0).start()

            @pl.when(jnp.logical_not(more))
            def _():
                for cp in ffn_copies(0, 0) + ffn_copies(1, 1):
                    cp.start()
            x_copy(hg, 1).start()
            st_copy(2, hg).wait()
            x_copy(hg, 0).wait()
            _weave(project_pre(1, h0, zero), relayout(2, sg * HC), *norm_and_score(hg, sg, 0, ln_cut, score))

            @pl.when(more)
            def _():
                st_copy(1, hg + 1).start()
                for j in range(1, NWO):
                    wo_copy(hg, j).start()
                st_copy(0, hg + 1).wait()
            x_copy(hg, 1).wait()
            _weave(project_pre(2, h0, zero), relayout(0, sg * HC + HC), *norm_and_score(hg, sg, ln_cut, XR, score))

            @pl.when(more)
            def _():
                st_copy(2, hg + 1).start()
                x_copy(hg + 1, 0).start()
                st_copy(1, hg + 1).wait()
                for j in range(NWO):
                    wo_copy(hg, j).wait()
                _weave(project_pre(0, h0 + HC), relayout(1, sg * HC + HC), repack_wo(sg))
            return score[0]

        score = jax.lax.fori_loop(0, NHG, pre_body, jnp.zeros((16, 128), F32))

        def first_max(key, free):
            top = jnp.max(jnp.max(key, axis=1, keepdims=True), axis=0, keepdims=True)
            first = jnp.where((key == top) & free, token, float(S))
            return top, jnp.min(jnp.min(first, axis=1, keepdims=True), axis=0, keepdims=True)

        token = (lane * 16 + sub).astype(F32)
        key = jnp.where(score == score, score, -jnp.inf)
        top1, i1 = first_max(key, token >= 0)
        top2, i2 = first_max(jnp.where(token == i1, -jnp.inf, key), token != i1)
        gate = jnp.where(sub == 0, _rnd(jax.nn.sigmoid(top1)), _rnd(jax.nn.sigmoid(top2)))
        picked = [i.astype(I32)[0, 0] for i in (i1, i2)]
        blocks = [pl.multiple_of(i & ~15, 16) for i in picked]
        xsel = jnp.zeros((16, D), F32)
        for c in range(2):
            block = normed(blocks[c] >> 6, blocks[c] & 63, 16).astype(F32)
            row = jnp.sum(jnp.where(sub == picked[c] - blocks[c], block, 0.0), axis=0, keepdims=True)
            xsel = jnp.where(sub == c, row, xsel)
        xsel = jnp.concatenate([xsel, xsel], axis=0).astype(BF16)

        def segment(first, t, mem):
            xs = normed(t, 0 if first else SEG, SEG)
            lhs = jnp.concatenate(
                [jnp.concatenate([mem, xs[:16].astype(F32)[8:]], axis=0).astype(BF16), xs[16:]], axis=0)
            out_rows = 32 if first else 48
            pending, probs, result = {}, {}, [None] * KD

            def pair_rows(m, g):
                return _rows(QKV0 + (m * (H // PAIR) + g) * GR, GR)

            def project(m, h):
                y = _dot(lhs, weight(m, h))
                pre = _halves(pre_v[t, m, h]).astype(F32)
                g, j = divmod(h, PAIR)
                pending.setdefault((m, g), []).extend([pre[:8] if first else pre[8:], y[M:], y[:M]])
                if j == PAIR - 1:
                    w_v[pair_rows(m, g), :] = _words(jnp.concatenate(pending.pop((m, g)), axis=0).astype(BF16))

            def score_pair(g):
                s = jax.lax.dot_general(_halves(w_v[pair_rows(0, g), :]), _halves(w_v[pair_rows(1, g), :]),
                                        CONTRACT_LAST, preferred_element_type=F32)
                fill = _floats(w_v[_rows(FILL0, PAIR * L), :])[:, :PAIR * L]
                s = jnp.where(fill == 0.0, s * scale, fill)
                e = jnp.exp(s - jnp.max(s, axis=-1, keepdims=True))
                probs[g] = (e * (1.0 / jnp.sum(e, axis=-1, keepdims=True))).astype(BF16)

            def mix(g):
                o = _dot(probs.pop(g), _halves(w_v[pair_rows(2, g), :]))
                for j in range(PAIR):
                    h, oh = g * PAIR + j, o[j * L:(j + 1) * L]
                    if first:
                        w_v[_rows(CO0 + h * 8, 8), :] = _words(oh[24:SEG])
                        oh = jnp.concatenate([oh[:24], oh[SEG:]], axis=0)
                    else:
                        oh = jnp.concatenate([_floats(w_v[_rows(CO0 + h * 8, 8), :]), oh], axis=0)
                    w_v[_rows(O0 + h * 24, out_rows // 2), :] = _words(oh.astype(BF16))

            def output(n, h0, h1):
                heads = jnp.concatenate([w_v[_rows(O0 + h * 24, out_rows // 2), :] for h in range(h0, h1)], axis=1)
                wo = w_v[_rows(WO0 + (n * H + h0) * (Dh // 2), (h1 - h0) * (Dh // 2)), :]
                y = _dot(_halves(heads), _halves(wo))
                if h0 > 0:
                    y = _floats(w_v[_rows(ACC0 + n * 48, out_rows), :]) + y
                if h1 < H:
                    w_v[_rows(ACC0 + n * 48, out_rows), :] = _words(y)
                else:
                    result[n] = y

            jobs = {"project": project, "score": score_pair, "mix": mix, "output": output}
            for name, *args in _plan(H, PAIR, KD, out_rows, PAIR * L, cuts, early, d_proj, d_soft, d_mix):
                jobs[name](*args)
            return jnp.concatenate(result, axis=1)

        def emit(t, r, n, attended):
            rows = pl.ds(pl.multiple_of(t * 64 + r, 16), n)
            out_v[rows, :] = (x_v[rows, :].astype(F32) + normed(t, r, n).astype(F32) + attended).astype(BF16)

        def two_segments(t, mem):
            slot = t % 2

            @pl.when(t < NF)
            def _():
                for cp in ffn_copies(t, slot):
                    cp.wait()
            ya = segment(True, t, mem)
            g = _rnd(_dot(xsel, wg_v[slot])[:16])
            u = _rnd(_dot(xsel, wu_v[slot])[:16])
            hid = jnp.where(t < NF, _rnd(g * _rnd(jax.nn.sigmoid(g))) * u, 0.0).astype(BF16)
            emit(t, 0, 16, ya[:16])
            yb = segment(False, t, ya[24:])
            y_v[...] += _dot(hid, wd_v[slot])
            emit(t, 16, 48, jnp.concatenate([ya[16:24], yb[:40]], axis=0))
            out_copy(t).start()

            @pl.when(t + 2 < NF)
            def _():
                for cp in ffn_copies(t + 2, slot):
                    cp.start()
            return yb[40:]

        jax.lax.fori_loop(0, NPASS, two_segments, mem0_v[0].astype(F32))

        sent = pl.ds(0, (NPASS - 1) * 64)
        pltpu.make_async_copy(out_v.at[sent, :], out_hbm.at[sent, :], sem_out.at[0]).wait()
        late = jnp.maximum(blocks[0], blocks[1]) >= (NPASS - 1) * 64

        @pl.when(late)
        def _():
            out_copy(NPASS - 1).wait()
        y = _rnd(_rnd(y_v[...]) * gate)
        for c in range(2):
            block = out_v[pl.ds(blocks[c], 16), :].astype(F32)
            out_v[pl.ds(blocks[c], 16), :] = jnp.where(
                sub == picked[c] - blocks[c], block + y[c:c + 1], block).astype(BF16)
        fix = [pltpu.make_async_copy(out_v.at[pl.ds(blocks[c], 16), :], out_hbm.at[pl.ds(blocks[c], 16), :],
                                     sem_fix.at[c]) for c in range(2)]
        fix[0].start()

        @pl.when(blocks[0] != blocks[1])
        def _():
            fix[1].start()
            fix[1].wait()

        @pl.when(jnp.logical_not(late))
        def _():
            out_copy(NPASS - 1).wait()
        fix[0].wait()

    scratch = [
        pltpu.VMEM((1, M, D), BF16),
        pltpu.VMEM((D,), BF16),
        pltpu.VMEM((S + 16, D), BF16),
        pltpu.VMEM((NSEG, 8, D), BF16),
        pltpu.VMEM((KD, NPRE // 2, 128), U32),
        pltpu.VMEM((3, D, HC, 128), BF16),
        pltpu.VMEM((FILL0 + PAIR * L, 128), U32),
        pltpu.VMEM((NWO, OR, D), BF16),
        pltpu.VMEM((NPASS, 3, H, 8, 128), U32),
        pltpu.VMEM((2, D, 128), BF16),
        pltpu.VMEM((2, D, 128), BF16),
        pltpu.VMEM((2, 128, D), BF16),
        pltpu.VMEM((16, D), F32),
        pltpu.VMEM((S, D), BF16),
        pltpu.SMEM((NHG,), I32),
        pltpu.SemaphoreType.DMA((2,)),
        pltpu.SemaphoreType.DMA((4,)),
        pltpu.SemaphoreType.DMA((4,)),
        pltpu.SemaphoreType.DMA((2,)),
        pltpu.SemaphoreType.DMA((3,)),
        pltpu.SemaphoreType.DMA((NWO,)),
        pltpu.SemaphoreType.DMA((6,)),
        pltpu.SemaphoreType.DMA((2,)),
        pltpu.SemaphoreType.DMA((2,)),
    ]
    return kernel, scratch


def run(A_x, A_mem0, A_Wq, A_Wk, A_Wv, A_Wo, A_seg_len, B_x, B_w_r, B_w_gate, B_w_up, B_w_down, **kw):
    del B_x
    B, S, D = A_x.shape
    _, H, Dh = A_Wq.shape
    seg = int(A_seg_len)
    assert B == 1
    kernel, scratch = make_kernel(S, D, H, Dh, A_mem0.shape[1], seg, B_w_gate.shape[1], **kw)
    hbm = pl.BlockSpec(memory_space=pl.ANY)
    out = pl.pallas_call(
        kernel,
        out_shape=jax.ShapeDtypeStruct((S, D), A_x.dtype),
        in_specs=[hbm] * 11,
        out_specs=hbm,
        scratch_shapes=scratch,
        compiler_params=pltpu.CompilerParams(vmem_limit_bytes=100 * 1024 * 1024, disable_bounds_checks=True),
    )(A_x.reshape(S, D), A_x.reshape(S // seg, seg, D), A_mem0, A_Wq, A_Wk, A_Wv,
      A_Wo.reshape(H * Dh, D), B_w_r, B_w_gate, B_w_up, B_w_down)
    return out.reshape(B, S, D)


@functools.partial(jax.jit, static_argnames=("A_seg_len",))
def pallas_parallel_sum__memory_aug_recurrent_mem_tr__moe_arch_mod__prompt_kernel(
    A_x, A_mem0, A_Wq, A_Wk, A_Wv, A_Wo, A_seg_len, B_x, B_w_r, B_w_gate, B_w_up, B_w_down,
):
    return run(A_x, A_mem0, A_Wq, A_Wk, A_Wv, A_Wo, A_seg_len, B_x, B_w_r, B_w_gate, B_w_up, B_w_down)
```
